```python
import jax
import jax.numpy as jnp

def _softmax(x, axis=-1):
    return jax.nn.softmax(x, axis=axis)

def _gelu(x):
    return jax.nn.gelu(x, approximate=True)

def _silu(x):
    return jax.nn.silu(x)

def _sigmoid(x):
    return jax.nn.sigmoid(x)

def _layernorm(x, axis=-1, eps=1e-05):
    m = jnp.mean(x, axis=axis, keepdims=True)
    v = jnp.var(x, axis=axis, keepdims=True)
    return (x - m) / jnp.sqrt(v + eps)

def _scatter_add(tgt, idx, src, axis=0):
    return tgt.at[idx].add(src)

def _segment_sum(src, seg, n):
    return jax.ops.segment_sum(src, seg, n)

class _Rng:

    def __init__(self, key):
        self._k = key

    def _next(self):
        self._k, sub = jax.random.split(self._k)
        return sub

    def normal(self, shape):
        return jax.random.normal(self._next(), shape, dtype=jnp.bfloat16)

    def randint(self, lo, hi, shape):
        return jax.random.randint(self._next(), shape, lo, hi, dtype=jnp.int32)

    def uniform(self, shape, lo=0.0, hi=1.0):
        return jax.random.uniform(self._next(), shape, jnp.bfloat16, lo, hi)

    def permutation(self, n):
        return jax.random.permutation(self._next(), n)
kernel_name = 'interleave_layers__linear_kernel_hedgehog__mixer_gmlp__prompt'

def _fwd_setup_inputs():
    _rng = _Rng(jax.random.key(int.from_bytes(__import__("os").urandom(4), "little")))
    _w = lambda a: (lambda t: t.astype(jnp.bfloat16) if jnp.issubdtype(t.dtype, jnp.floating) else t)(jnp.asarray(a))

    def _A_setup():
        B, S, D, H = (1, 2048, 640, 32)
        Dh = D // H
        return {'x': _w((lambda *s: _rng.normal(s) * 0.05)(B, S, D)), 'wqkv': _w((lambda *s: _rng.normal(s) * 0.05)(D, 3 * D)), 'w_phi': _w((lambda *s: _rng.normal(s) * 0.05)(H, Dh, Dh) * Dh ** (-0.5)), 'wo': _w((lambda *s: _rng.normal(s) * 0.05)(D, D))}
    _A_in = _A_setup()

    def _B_setup():
        B, S, D, F = (1, 2048, 640, 1536)
        Fh = F // 2
        return {'x': _w((lambda *s: _rng.normal(s) * 0.05)(B, S, D)), 'w_in': _w((lambda *s: _rng.normal(s) * 0.05)(D, 2 * Fh)), 'w_sp': _w(0.01 * (lambda *s: _rng.normal(s) * 0.05)(S, S)), 'b_sp': _w(1.0 + 0.01 * (lambda *s: _rng.normal(s) * 0.05)(S)), 'w_out': _w((lambda *s: _rng.normal(s) * 0.05)(Fh, D))}
    _B_in = _B_setup()
    return {'A_x': _A_in['x'], 'A_wqkv': _A_in['wqkv'], 'A_w_phi': _A_in['w_phi'], 'A_wo': _A_in['wo'], 'B_x': _B_in['x'], 'B_w_in': _B_in['w_in'], 'B_w_sp': _B_in['w_sp'], 'B_b_sp': _B_in['b_sp'], 'B_w_out': _B_in['w_out']}

def _fwd_reference(A_x, A_wqkv, A_w_phi, A_wo, B_x, B_w_in, B_w_sp, B_b_sp, B_w_out):

    def _A_ref(x, wqkv, w_phi, wo):
        B, S, D = x.shape
        H = 32
        Dh = D // H
        qkv = (lambda x, *d: x.transpose(*d))((x @ wqkv).reshape(B, S, 3, H, Dh), 2, 0, 3, 1, 4)
        q, k, v = (qkv[0], qkv[1], qkv[2])
        pq = jnp.einsum('bhsd,hdf->bhsf', q, w_phi)
        pk = jnp.einsum('bhsd,hdf->bhsf', k, w_phi)
        phi_q = jnp.concatenate([_softmax(pq, axis=-1), _softmax(-pq, axis=-1)], axis=-1)
        phi_k = jnp.concatenate([_softmax(pk, axis=-1), _softmax(-pk, axis=-1)], axis=-1)
        kv = jnp.einsum('bhsf,bhsd->bhfd', phi_k, v)
        z = jnp.einsum('bhsf->bhf', phi_k)
        num = jnp.einsum('bhqf,bhfd->bhqd', phi_q, kv)
        den = jnp.einsum('bhqf,bhf->bhq', phi_q, z)[..., None] + 1e-06
        o = num / den
        return (lambda x, *d: x.transpose(*d))(o, 0, 2, 1, 3).reshape(B, S, D) @ wo

    def _B_ref(x, w_in, w_sp, b_sp, w_out):
        B, S, D = x.shape
        F = w_in.shape[-1]
        Fh = F // 2
        z = _gelu(jnp.einsum('bsd,df->bsf', x, w_in))
        z1 = z[..., :Fh].copy()
        z2 = _layernorm(z[..., Fh:], axis=-1)
        g = jnp.einsum('ts,bsf->btf', w_sp, z2) + b_sp[None, :, None]
        return jnp.einsum('bsf,fd->bsd', z1 * g, w_out)
    x = A_x
    x = x + _A_ref(_layernorm(x, axis=-1), A_wqkv, A_w_phi, A_wo)
    x = x + _B_ref(_layernorm(x, axis=-1), B_w_in, B_w_sp, B_b_sp, B_w_out)
    x = x + _A_ref(_layernorm(x, axis=-1), A_wqkv, A_w_phi, A_wo)
    x = x + _B_ref(_layernorm(x, axis=-1), B_w_in, B_w_sp, B_b_sp, B_w_out)
    return x

def setup_inputs():
    _inp = _fwd_setup_inputs()
    _gk = jax.random.fold_in(jax.random.key(int.from_bytes(__import__("os").urandom(4), "little")), 2 ** 31 - 1)
    _shapes = [[1, 2048, 640]]
    _dtypes = ['bfloat16']
    _gks = jax.random.split(_gk, len(_shapes))
    _gs = [jax.random.normal(k, s, dtype=jnp.dtype(d)) * 0.05 for k, s, d in zip(_gks, _shapes, _dtypes)]
    _inp['grad_out'] = _gs[0]
    return _inp

def reference(A_x, A_wqkv, A_w_phi, A_wo, B_w_in, B_w_sp, B_b_sp, B_w_out, B_x, grad_out):
    _const = dict(B_x=B_x)

    def _f(*_d):
        return _fwd_reference(**{'A_x': _d[0], 'A_wqkv': _d[1], 'A_w_phi': _d[2], 'A_wo': _d[3], 'B_w_in': _d[4], 'B_w_sp': _d[5], 'B_b_sp': _d[6], 'B_w_out': _d[7], **_const})
    _out, _vjp = jax.vjp(_f, A_x, A_wqkv, A_w_phi, A_wo, B_w_in, B_w_sp, B_b_sp, B_w_out)
    _grads = _vjp(grad_out)
    _out0 = jnp.asarray(_out)
    return (_out0, *[jnp.asarray(_g) for _g in _grads])
```

```python
import functools
import math

import jax
import jax.numpy as jnp
from jax import lax
import jax.experimental.pallas as pl
import jax.experimental.pallas.tpu as pltpu

S = 2048
D = 640
H = 32
DH = 20
F2 = 1536
FH = 768
NG = 4
GR = 160
GF = 320
KS = (0, 128, 256, 384)
RR = ((0, 160), (0, 320), (160, 480), (320, 640), (480, 640))
TM = 256
NB = S // TM
EPS_LN = 1e-5
EPS_DEN = 1e-6
GELU_C = math.sqrt(2.0 / math.pi)
GELU_A = 0.044715

F32 = jnp.float32
BF16 = jnp.bfloat16


def _dot(a, b):
    return jnp.dot(a, b, preferred_element_type=F32)


def _dot_nt(a, b):
    return lax.dot_general(a, b, (((1,), (1,)), ((), ())), preferred_element_type=F32)


def _dot_tn(a, b):
    return lax.dot_general(a, b, (((0,), (0,)), ((), ())), preferred_element_type=F32)


def _ln(x):
    m = jnp.mean(x, axis=-1, keepdims=True)
    xc = x - m
    v = jnp.mean(xc * xc, axis=-1, keepdims=True)
    r = lax.rsqrt(v + EPS_LN)
    return xc * r, r


def _ln_bwd(dy, xn, r):
    a = jnp.mean(dy, axis=-1, keepdims=True)
    b = jnp.mean(dy * xn, axis=-1, keepdims=True)
    return r * (dy - a - xn * b)


def _iota(shape, dim):
    return lax.broadcasted_iota(jnp.int32, shape, dim)


def _row_map(r):
    g = ((r >= GR).astype(jnp.int32) + (r >= 2 * GR).astype(jnp.int32)
         + (r >= 3 * GR).astype(jnp.int32))
    rem = r - GR * g
    return rem >> 3, 8 * g + (rem & 7)


def _tile(r, n):
    return jnp.concatenate([r] * n, axis=1)


def _phi_t(pt):
    p4 = pt.reshape(NG, DH, 8, pt.shape[1])
    mx = jnp.max(p4, axis=1, keepdims=True)
    mn = jnp.min(p4, axis=1, keepdims=True)
    ep = jnp.exp(p4 - mx)
    en = jnp.exp(mn - p4)
    sp = jnp.sum(ep, axis=1, keepdims=True)
    sn = jnp.sum(en, axis=1, keepdims=True)
    return ep * (1.0 / sp), en * (1.0 / sn)


def _phi_bwd_t(php, phn, dphp, dphn):
    cp = jnp.sum(dphp * php, axis=1, keepdims=True)
    cn = jnp.sum(dphn * phn, axis=1, keepdims=True)
    return php * (dphp - cp) - phn * (dphn - cn)


def _rbf(x):
    return x.astype(BF16).astype(F32)


def _gelu(u):
    t = jnp.tanh(GELU_C * (u + GELU_A * (u * u * u)))
    return 0.5 * u * (1.0 + t)


def _gelu_and_grad(u):
    u2 = u * u
    t = jnp.tanh(GELU_C * (u + GELU_A * (u2 * u)))
    a = 0.5 * u * (1.0 + t)
    da = 0.5 * (1.0 + t) + 0.5 * u * (1.0 - t * t) * (GELU_C * (1.0 + 3.0 * GELU_A * u2))
    return a, da


def _kernel(
    x_hbm, wqkv_hbm, wphi_hbm, wo_hbm, win_hbm, wsp_hbm, bsp_hbm, wout_hbm, gout_hbm,
    out_hbm, dx_hbm, dwqkv_hbm, dwphi_hbm, dwo_hbm, dwin_hbm, dwsp_hbm, dbsp_hbm, dwout_hbm,
    sp_pq, sp_pk, sp_v, sp_o, sp_u, sp_g,
    xs_ref,
    hs_ref,
    rs_ref,
    gout_ref,
    dx_ref,
    pq_ref, pk_ref, v_ref, o_ref,
    u_ref,
    g_ref,
    z2_ref,
    dg_ref,
    wqkv_ref,
    wphi_ref,
    wo_ref,
    win_ref,
    wsp_ref,
    bsp_ref,
    wout_ref,
    wp_ref,
    phip_ref,
    pmt_ref,
    wop_ref,
    bcol_ref,
    dwp_ref,
    dwo_acc,
    dwin_acc,
    dwout_acc,
    kv_acc,
    kvm_ref,
    kvt_ref,
    dkvm_ref,
    dkvt_ref,
    zacc_ref,
    z_ref,
    dz_ref,
    ostage,
    wspstage,
    dbstage,
    dwphi_stage,
    sem_in, sem_spill, sem_rest, sem_out, sem_blk,
):
    def rows(i):
        if isinstance(i, int):
            return pl.ds(i * TM, TM)
        return pl.ds(pl.multiple_of(i * TM, TM), TM)

    wq_copies = [
        pltpu.make_async_copy(wqkv_hbm.at[:, t * D:(t + 1) * D], wqkv_ref.at[:, t * D:(t + 1) * D],
                              sem_in.at[9 + t])
        for t in range(3)
    ]
    pltpu.make_async_copy(wphi_hbm, wphi_ref, sem_in.at[2]).start()
    for c in wq_copies:
        c.start()
    in_copies = [
        pltpu.make_async_copy(x_hbm.at[0], xs_ref.at[0], sem_in.at[0]),
        None,
        None,
        pltpu.make_async_copy(wo_hbm, wo_ref, sem_in.at[3]),
        pltpu.make_async_copy(win_hbm, win_ref, sem_in.at[4]),
        pltpu.make_async_copy(bsp_hbm, bsp_ref, sem_in.at[5]),
        pltpu.make_async_copy(wsp_hbm, wsp_ref, sem_in.at[6]),
        pltpu.make_async_copy(wout_hbm, wout_ref, sem_in.at[7]),
        pltpu.make_async_copy(gout_hbm.at[0], gout_ref, sem_in.at[8]),
    ]
    for c in in_copies:
        if c is not None:
            c.start()

    def pmt_mat():
        f, head = _row_map(_iota((D, D), 0))
        return (_iota((D, D), 1) == head * DH + f).astype(BF16)

    def head_mask():
        c_dd = _iota((D, D), 1)
        _, head = _row_map(_iota((D, D), 0))
        hc = head * DH
        return jnp.logical_and(c_dd >= hc, c_dd < hc + DH)

    def et_mat():
        f, _ = _row_map(_iota((D, DH), 0))
        return (_iota((D, DH), 1) == f).astype(BF16)

    with jax.named_scope("prep"):
        dwp_ref[...] = jnp.zeros_like(dwp_ref)
        dwo_acc[...] = jnp.zeros_like(dwo_acc)
        dwin_acc[...] = jnp.zeros_like(dwin_acc)
        dwout_acc[...] = jnp.zeros_like(dwout_acc)
        pltpu.make_async_copy(wphi_hbm, wphi_ref, sem_in.at[2]).wait()
        phip_ref[...] = jnp.where(head_mask(), _dot_nt(et_mat(), wphi_ref[...]), 0.0).astype(BF16)
        pmt_ref[...] = pmt_mat()
        for t in range(3):
            wq_copies[t].wait()
            m_ref = phip_ref if t < 2 else pmt_ref
            for g in range(NG):
                wp_ref[t * D + g * GR:t * D + (g + 1) * GR, :] = _dot_nt(
                    m_ref[g * GR:(g + 1) * GR, KS[g]:KS[g] + 256],
                    wqkv_ref[:, t * D + KS[g]:t * D + KS[g] + 256]).astype(BF16)
        in_copies[3].wait()
        for g in range(NG):
            wop_ref[g * GR:(g + 1) * GR, :] = _dot(
                pmt_ref[g * GR:(g + 1) * GR, KS[g]:KS[g] + 256],
                wo_ref[KS[g]:KS[g] + 256, :]).astype(BF16)

    def kv_finish(m_ref, t_ref, off):
        mask = (_iota((384, 256), 0) & 7) == (_iota((384, 256), 1) & 7)
        for g in range(NG):
            m = jnp.where(mask, kv_acc[g], 0.0)
            m_ref[off + g] = m[0:GF, 0:GR].astype(BF16)
            t_ref[off + g] = jnp.transpose(m)[0:GR, 0:GF].astype(BF16)

    def z_finish():
        zs = jnp.sum(zacc_ref[...], axis=1, keepdims=True)
        return jnp.broadcast_to(zs, (2 * D, 128))

    def z4(zval):
        return _tile(zval, TM // 128).reshape(NG, 2 * DH, 8, TM)

    def fold_lanes(x):
        x2 = x.reshape(2 * D, TM)
        r = x2[:, 0:128]
        for j in range(1, TM // 128):
            r = r + x2[:, 128 * j:128 * (j + 1)]
        return r

    spill_bufs = [(pq_ref, sp_pq), (pk_ref, sp_pk), (v_ref, sp_v), (o_ref, sp_o),
                  (u_ref, sp_u), (g_ref, sp_g)]

    def spill_copy(k, i):
        src, dst = spill_bufs[k]
        idx = i if k < 4 else rows(i)
        return pltpu.make_async_copy(src.at[idx], dst.at[idx], sem_spill.at[k * NB + i])

    def spill_wait(k):
        for i in range(NB):
            spill_copy(k, i).wait()

    def restore_copy(k):
        dst, src = spill_bufs[k]
        return pltpu.make_async_copy(src, dst, sem_rest.at[k])

    def restore_u_copy(i):
        return pltpu.make_async_copy(sp_u.at[rows(i)], u_ref.at[rows(i)], sem_blk.at[i])

    def a_fwd1(layer, i):
        x = xs_ref[0, rows(i), :].astype(F32)
        xn, r = _ln(x)
        h = xn.astype(BF16)
        hs_ref[2 * layer, rows(i), :] = h
        rs_ref[2 * layer, rows(i), :] = r
        pt = _dot_nt(wp_ref[...], h)
        pq = pt[0:D].astype(BF16)
        pk = pt[D:2 * D].astype(BF16)
        v = pt[2 * D:3 * D].astype(BF16)
        pq_ref[i] = pq
        pk_ref[i] = pk
        v_ref[i] = v
        if layer == 0:
            for k in range(3):
                spill_copy(k, i).start()
        kp, kn = _phi_t(pk.astype(F32))
        phik = jnp.concatenate([kp, kn], axis=1).astype(BF16)
        for g in range(NG):
            kv_acc[g, 0:GF, 0:GR] += _dot_nt(phik[g].reshape(GF, TM), v[g * GR:(g + 1) * GR])
        zacc_ref[...] += fold_lanes(phik.astype(F32))

    def a_fwd_finish(layer):
        kv_finish(kvm_ref, kvt_ref, layer * NG)
        z_ref[layer] = z_finish()

    def a_fwd2(layer, i):
        x = xs_ref[0, rows(i), :].astype(F32)
        qp, qn = _phi_t(pq_ref[i].astype(F32))
        phiq = jnp.concatenate([qp, qn], axis=1).astype(BF16)
        num = jnp.concatenate(
            [_dot(kvt_ref[layer * NG + g], phiq[g].reshape(GF, TM)) for g in range(NG)], axis=0)
        den = jnp.sum(phiq.astype(F32) * z4(z_ref[layer]), axis=1, keepdims=True) + EPS_DEN
        o = (num.reshape(NG, DH, 8, TM) * (1.0 / den)).reshape(D, TM).astype(BF16)
        o_ref[i] = o
        if layer == 0:
            spill_copy(3, i).start()
        x1 = (x + _dot_tn(o, wop_ref[...])).astype(BF16)
        xs_ref[1, rows(i), :] = x1
        return x1

    def b_fwd1(layer, i, x1):
        xn, r = _ln(x1.astype(F32))
        h = xn.astype(BF16)
        hs_ref[2 * layer + 1, rows(i), :] = h
        rs_ref[2 * layer + 1, rows(i), :] = r
        u = _dot(h, win_ref[...]).astype(BF16)
        u_ref[rows(i), :] = u
        if layer == 0:
            spill_copy(4, i).start()
        a2 = _gelu(u[:, FH:F2].astype(F32))
        z2, _ = _ln(a2)
        z2_ref[rows(i), layer * FH:(layer + 1) * FH] = z2.astype(BF16)

    def b_fwd2(layer, i):
        x1 = xs_ref[1, rows(i), :].astype(F32)
        g = _dot(wsp_ref[rows(i), :], z2_ref[:, layer * FH:(layer + 1) * FH])
        g = (g + _tile(bcol_ref[rows(i), :], FH // 128)).astype(BF16)
        g_ref[rows(i), :] = g
        if layer == 0:
            spill_copy(5, i).start()
        z1 = _gelu(u_ref[rows(i), 0:FH].astype(F32))
        y = (z1 * g.astype(F32)).astype(BF16)
        x2 = (x1 + _dot(y, wout_ref[...])).astype(BF16)
        return x2

    def b_bwd1(layer, i, dy):
        dyb = dy.astype(BF16)
        g = g_ref[rows(i), :].astype(F32)
        z1, dgelu1 = _gelu_and_grad(u_ref[rows(i), 0:FH].astype(F32))
        y = (z1 * g).astype(BF16)
        dzg = _dot_nt(dyb, wout_ref[...])
        dwout_acc[...] += _dot_tn(y, dyb)
        dg = (dzg * z1).astype(BF16)
        dg_ref[rows(i), layer * FH:(layer + 1) * FH] = dg
        du1 = (dzg * g * dgelu1).astype(BF16)
        h = hs_ref[2 * layer + 1, rows(i), :]
        gout_ref[rows(i), :] = _dot_nt(du1, win_ref[:, 0:FH]).astype(BF16)
        dwin_acc[:, 0:FH] += _dot_tn(h, du1)

    def b_bwd2(layer, i, dxp):
        dz2 = _dot_tn(wsp_ref[:, rows(i)], dg_ref[:, layer * FH:(layer + 1) * FH])
        a2, dgelu2 = _gelu_and_grad(u_ref[rows(i), FH:F2].astype(F32))
        z2n, r2 = _ln(a2)
        du2 = (_ln_bwd(dz2, z2n, r2) * dgelu2).astype(BF16)
        h = hs_ref[2 * layer + 1, rows(i), :]
        dh = _dot_nt(du2, win_ref[:, FH:F2]) + gout_ref[rows(i), :].astype(F32)
        dwin_acc[:, FH:F2] += _dot_tn(h, du2)
        return dxp + _ln_bwd(dh, h.astype(F32), rs_ref[2 * layer + 1, rows(i), :])

    def a_bwd1(layer, i, dy):
        dyb = dy.astype(BF16)
        ob = o_ref[i]
        do = _dot_nt(wop_ref[...], dyb).reshape(NG, DH, 8, TM)
        dwo_acc[...] += _dot(ob, dyb)
        qp, qn = _phi_t(pq_ref[i].astype(F32))
        qp = _rbf(qp)
        qn = _rbf(qn)
        phiq_f = jnp.concatenate([qp, qn], axis=1)
        phiq = phiq_f.astype(BF16)
        z = z4(z_ref[layer])
        rden = 1.0 / (jnp.sum(phiq_f * z, axis=1, keepdims=True) + EPS_DEN)
        dnum = (do * rden).astype(BF16)
        dden = -jnp.sum(do * ob.astype(F32).reshape(NG, DH, 8, TM), axis=1, keepdims=True) * rden
        dphi = []
        for g in range(NG):
            dn = dnum[g].reshape(GR, TM)
            dphi.append(_dot(kvm_ref[layer * NG + g], dn))
            kv_acc[g, 0:GF, 0:GR] += _dot_nt(phiq[g].reshape(GF, TM), dn)
        dphi = jnp.concatenate(dphi, axis=0).reshape(NG, 2 * DH, 8, TM) + dden * z
        zacc_ref[...] += fold_lanes(phiq_f * dden)
        dpq = _phi_bwd_t(qp, qn, dphi[:, 0:DH], dphi[:, DH:2 * DH]).reshape(D, TM).astype(BF16)
        h = hs_ref[2 * layer, rows(i), :]
        gout_ref[rows(i), :] = _dot_tn(dpq, wp_ref[0:D, :]).astype(BF16)
        dwp_ref[0:D, :] += _dot(dpq, h)

    def a_bwd_finish():
        kv_finish(dkvm_ref, dkvt_ref, 0)
        dz_ref[...] = z_finish()

    def a_bwd2(layer, i, dxp):
        v = v_ref[i]
        kp, kn = _phi_t(pk_ref[i].astype(F32))
        kp = _rbf(kp)
        kn = _rbf(kn)
        phik = jnp.concatenate([kp, kn], axis=1).astype(BF16)
        dphi, dvs = [], []
        for g in range(NG):
            dphi.append(_dot(dkvm_ref[g], v[g * GR:(g + 1) * GR]))
            dvs.append(_dot(dkvt_ref[g], phik[g].reshape(GF, TM)))
        dphi = jnp.concatenate(dphi, axis=0).reshape(NG, 2 * DH, 8, TM) + z4(dz_ref[...])
        dpk = _phi_bwd_t(kp, kn, dphi[:, 0:DH], dphi[:, DH:2 * DH]).reshape(D, TM)
        dkv = jnp.concatenate([dpk] + dvs, axis=0).astype(BF16)
        h = hs_ref[2 * layer, rows(i), :]
        dh = _dot_tn(dkv, wp_ref[D:3 * D, :]) + gout_ref[rows(i), :].astype(F32)
        dwp_ref[D:3 * D, :] += _dot(dkv, h)
        return dxp + _ln_bwd(dh, h.astype(F32), rs_ref[2 * layer, rows(i), :])

    def loop(body, name="loop", unroll=1):
        def b(i, c):
            for k in range(unroll):
                body(i * unroll + k)
            return c
        with jax.named_scope(name):
            lax.fori_loop(0, NB // unroll, b, 0)

    def stage_out(i, val, dst_hbm, stage, semoff):
        slot = i % 2

        @pl.when(i >= 2)
        def _():
            pltpu.make_async_copy(stage.at[slot], dst_hbm.at[rows(i - 2)],
                                  sem_blk.at[semoff + slot]).wait()
        stage[slot] = val
        pltpu.make_async_copy(stage.at[slot], dst_hbm.at[rows(i)], sem_blk.at[semoff + slot]).start()

    def stage_drain(dst_hbm, stage, semoff):
        for i in (NB - 2, NB - 1):
            slot = i % 2
            pltpu.make_async_copy(stage.at[slot], dst_hbm.at[rows(i)],
                                  sem_blk.at[semoff + slot]).wait()

    with jax.named_scope("pre1"):
        in_copies[0].wait()
        kv_acc[...] = jnp.zeros_like(kv_acc)
        zacc_ref[...] = jnp.zeros_like(zacc_ref)
    loop(lambda i: a_fwd1(0, i), "P1", 2)

    with jax.named_scope("pre2"):
        a_fwd_finish(0)
        in_copies[4].wait()
        in_copies[5].wait()
        bcol_ref[...] = jnp.transpose(
            jnp.broadcast_to(bsp_ref[...].astype(F32), (128, S)))

    def p2(layer, name):
        with jax.named_scope(name):
            a_fwd2(layer, 0)

            def body(i, c):
                x1 = xs_ref[1, rows(i), :]
                a_fwd2(layer, i + 1)
                b_fwd1(layer, i, x1)
                return c
            lax.fori_loop(0, NB - 1, body, 0)
            b_fwd1(layer, NB - 1, xs_ref[1, rows(NB - 1), :])
    p2(0, "P2")

    with jax.named_scope("pre3"):
        in_copies[6].wait()
        in_copies[7].wait()
        for k in range(3):
            spill_wait(k)
        kv_acc[...] = jnp.zeros_like(kv_acc)
        zacc_ref[...] = jnp.zeros_like(zacc_ref)

    with jax.named_scope("P3"):
        xs_ref[0, rows(0), :] = b_fwd2(0, 0)

        def p3(i, c):
            x2 = b_fwd2(0, i + 1)
            a_fwd1(1, i)
            xs_ref[0, rows(i + 1), :] = x2
            return c
        lax.fori_loop(0, NB - 1, p3, 0)
        a_fwd1(1, NB - 1)

    with jax.named_scope("pre4"):
        a_fwd_finish(1)
        spill_wait(3)
        spill_wait(4)
    p2(1, "P4")

    with jax.named_scope("pre5"):
        spill_wait(5)
        in_copies[8].wait()

    def p5(i):
        x4 = b_fwd2(1, i)
        stage_out(i, x4, out_hbm.at[0], ostage, NB)
        dy = gout_ref[rows(i), :].astype(F32)
        dx_ref[rows(i), :] = dy
        b_bwd1(1, i, dy)
    loop(p5, "P5", 2)

    with jax.named_scope("pre6"):
        stage_drain(out_hbm.at[0], ostage, NB)
        restore_copy(5).start()
        kv_acc[...] = jnp.zeros_like(kv_acc)
        zacc_ref[...] = jnp.zeros_like(zacc_ref)

    def p6(layer, name):
        with jax.named_scope(name):
            dx_ref[rows(0), :] = b_bwd2(layer, 0, dx_ref[rows(0), :])
            if layer == 1:
                restore_u_copy(0).start()

            def body(i, c):
                dxa = dx_ref[rows(i), :]
                dxb = dx_ref[rows(i + 1), :]
                nb = b_bwd2(layer, i + 1, dxb)
                a_bwd1(layer, i, dxa)
                dx_ref[rows(i + 1), :] = nb
                if layer == 1:
                    restore_u_copy(i + 1).start()
                return c
            lax.fori_loop(0, NB - 1, body, 0)
            a_bwd1(layer, NB - 1, dx_ref[rows(NB - 1), :])
    p6(1, "P6")

    with jax.named_scope("pre7"):
        a_bwd_finish()
        restore_copy(0).start()
        restore_copy(3).start()
        restore_copy(5).wait()
        for i in range(NB):
            restore_u_copy(i).wait()

    def p7(i):
        dx2 = a_bwd2(1, i, dx_ref[rows(i), :])
        dx_ref[rows(i), :] = dx2
        b_bwd1(0, i, dx2)
    loop(p7, "P7")

    db_copy = pltpu.make_async_copy(dbstage, dbsp_hbm, sem_out.at[0])
    with jax.named_scope("pre8"):
        restore_copy(1).start()
        restore_copy(2).start()
        restore_copy(0).wait()
        restore_copy(3).wait()
        kv_acc[...] = jnp.zeros_like(kv_acc)
        zacc_ref[...] = jnp.zeros_like(zacc_ref)
    p6(0, "P8")

    dwin_copy = pltpu.make_async_copy(win_ref, dwin_hbm, sem_out.at[1])
    dwout_copy = pltpu.make_async_copy(wout_ref, dwout_hbm, sem_out.at[2])
    dwo_copy = pltpu.make_async_copy(wo_ref, dwo_hbm, sem_out.at[3])
    with jax.named_scope("pre9"):
        a_bwd_finish()
        win_ref[...] = dwin_acc[...].astype(BF16)
        dwin_copy.start()
        wout_ref[...] = dwout_acc[...].astype(BF16)
        dwout_copy.start()
        wop_ref[...] = dwo_acc[...].astype(BF16)
        for j in range(5):
            r0, r1 = RR[j]
            wo_ref[128 * j:128 * (j + 1), :] = _dot_tn(
                pmt_ref[r0:r1, 128 * j:128 * (j + 1)], wop_ref[r0:r1, :]).astype(BF16)
        dwo_copy.start()
        restore_copy(1).wait()
        restore_copy(2).wait()

    def p9(i):
        dgb = dg_ref[rows(i), :]
        dwsp = _dot_nt(dgb, z2_ref[...]).astype(BF16)
        db = _dot_nt(jnp.ones((8, 2 * FH), BF16), dgb)
        dx0 = a_bwd2(0, i, dx_ref[rows(i), :])
        stage_out(i, dwsp, dwsp_hbm, wspstage, NB + 2)
        dbstage[:, pl.ds(pl.multiple_of(i * TM, TM), TM)] = db[0:1, :].astype(BF16)
        stage_out(i, dx0.astype(BF16), dx_hbm.at[0], ostage, NB)
    loop(p9, "P9")

    dwqkv_copy = pltpu.make_async_copy(wqkv_ref, dwqkv_hbm, sem_out.at[4])
    dwphi_copy = pltpu.make_async_copy(dwphi_stage, dwphi_hbm, sem_out.at[5])
    with jax.named_scope("final"):
        db_copy.start()
        wp_ref[...] = dwp_ref[...].astype(BF16)
        dwo_acc[...] = jnp.zeros_like(dwo_acc)
        for g in range(NG):
            dwo_acc[g * GR:(g + 1) * GR, KS[g]:KS[g] + 256] = (
                _dot(wp_ref[g * GR:(g + 1) * GR, :], wqkv_ref[:, KS[g]:KS[g] + 256])
                + _dot(wp_ref[D + g * GR:D + (g + 1) * GR, :],
                       wqkv_ref[:, D + KS[g]:D + KS[g] + 256]))
        mm = jnp.where(head_mask(), dwo_acc[...], 0.0)
        mhi = mm.astype(BF16)
        mlo = (mm - mhi.astype(F32)).astype(BF16)
        dwphi_stage[...] = (_dot_tn(mhi, et_mat()) + _dot_tn(mlo, et_mat())).astype(BF16)
        dwphi_copy.start()
        for t in range(3):
            m_ref = phip_ref if t < 2 else pmt_ref
            for j in range(5):
                r0, r1 = RR[j]
                wqkv_ref[:, t * D + 128 * j:t * D + 128 * (j + 1)] = _dot_tn(
                    wp_ref[t * D + r0:t * D + r1, :],
                    m_ref[r0:r1, 128 * j:128 * (j + 1)]).astype(BF16)
        dwqkv_copy.start()

    with jax.named_scope("drain"):
        stage_drain(dwsp_hbm, wspstage, NB + 2)
        stage_drain(dx_hbm.at[0], ostage, NB)
        db_copy.wait()
        dwin_copy.wait()
        dwout_copy.wait()
        dwo_copy.wait()
        dwqkv_copy.wait()
        dwphi_copy.wait()


@jax.jit
def pallas_interleave_layers__linear_kernel_hedgehog__mixer_gmlp__prompt_kernel(
    A_x: jax.Array,
    A_wqkv: jax.Array,
    A_w_phi: jax.Array,
    A_wo: jax.Array,
    B_x: jax.Array,
    B_w_in: jax.Array,
    B_w_sp: jax.Array,
    B_b_sp: jax.Array,
    B_w_out: jax.Array,
    grad_out: jax.Array,
):
    del B_x
    wphi2d = A_w_phi.reshape(D, DH)
    bsp2d = B_b_sp.reshape(1, S)

    any_spec = pl.BlockSpec(memory_space=pl.ANY)
    out_shape = (
        jax.ShapeDtypeStruct((1, S, D), BF16),
        jax.ShapeDtypeStruct((1, S, D), BF16),
        jax.ShapeDtypeStruct((D, 3 * D), BF16),
        jax.ShapeDtypeStruct((D, DH), BF16),
        jax.ShapeDtypeStruct((D, D), BF16),
        jax.ShapeDtypeStruct((D, F2), BF16),
        jax.ShapeDtypeStruct((S, S), BF16),
        jax.ShapeDtypeStruct((1, S), BF16),
        jax.ShapeDtypeStruct((FH, D), BF16),
        jax.ShapeDtypeStruct((NB, D, TM), BF16),
        jax.ShapeDtypeStruct((NB, D, TM), BF16),
        jax.ShapeDtypeStruct((NB, D, TM), BF16),
        jax.ShapeDtypeStruct((NB, D, TM), BF16),
        jax.ShapeDtypeStruct((S, F2), BF16),
        jax.ShapeDtypeStruct((S, FH), BF16),
    )
    scratch_shapes = [
        pltpu.VMEM((2, S, D), BF16),
        pltpu.VMEM((4, S, D), BF16),
        pltpu.VMEM((4, S, 1), F32),
        pltpu.VMEM((S, D), BF16),
        pltpu.VMEM((S, D), F32),
        pltpu.VMEM((NB, D, TM), BF16),
        pltpu.VMEM((NB, D, TM), BF16),
        pltpu.VMEM((NB, D, TM), BF16),
        pltpu.VMEM((NB, D, TM), BF16),
        pltpu.VMEM((S, F2), BF16),
        pltpu.VMEM((S, FH), BF16),
        pltpu.VMEM((S, 2 * FH), BF16),
        pltpu.VMEM((S, 2 * FH), BF16),
        pltpu.VMEM((D, 3 * D), BF16),
        pltpu.VMEM((D, DH), BF16),
        pltpu.VMEM((D, D), BF16),
        pltpu.VMEM((D, F2), BF16),
        pltpu.VMEM((S, S), BF16),
        pltpu.VMEM((1, S), BF16),
        pltpu.VMEM((FH, D), BF16),
        pltpu.VMEM((3 * D, D), BF16),
        pltpu.VMEM((D, D), BF16),
        pltpu.VMEM((D, D), BF16),
        pltpu.VMEM((D, D), BF16),
        pltpu.VMEM((S, 128), F32),
        pltpu.VMEM((3 * D, D), F32),
        pltpu.VMEM((D, D), F32),
        pltpu.VMEM((D, F2), F32),
        pltpu.VMEM((FH, D), F32),
        pltpu.VMEM((NG, 384, 256), F32),
        pltpu.VMEM((2 * NG, GF, GR), BF16),
        pltpu.VMEM((2 * NG, GR, GF), BF16),
        pltpu.VMEM((NG, GF, GR), BF16),
        pltpu.VMEM((NG, GR, GF), BF16),
        pltpu.VMEM((2 * D, 128), F32),
        pltpu.VMEM((2, 2 * D, 128), F32),
        pltpu.VMEM((2 * D, 128), F32),
        pltpu.VMEM((2, TM, D), BF16),
        pltpu.VMEM((2, TM, S), BF16),
        pltpu.VMEM((1, S), BF16),
        pltpu.VMEM((D, DH), BF16),
        pltpu.SemaphoreType.DMA((12,)),
        pltpu.SemaphoreType.DMA((6 * NB,)),
        pltpu.SemaphoreType.DMA((6,)),
        pltpu.SemaphoreType.DMA((6,)),
        pltpu.SemaphoreType.DMA((NB + 4,)),
    ]
    outs = pl.pallas_call(
        _kernel,
        out_shape=out_shape,
        in_specs=[any_spec] * 9,
        out_specs=tuple([any_spec] * len(out_shape)),
        scratch_shapes=scratch_shapes,
        compiler_params=pltpu.CompilerParams(
            vmem_limit_bytes=125 * 1024 * 1024,
        ),
    )(A_x, A_wqkv, wphi2d, A_wo, B_w_in, B_w_sp, bsp2d, B_w_out, grad_out)
    out, dx0, dwqkv, dwphi, dwo, dwin, dwsp, dbsp, dwout = outs[:9]
    return (out, dx0, dwqkv, dwphi.reshape(H, DH, DH), dwo, dwin, dwsp,
            dbsp.reshape(S), dwout)
```

```python
import math

import jax
import jax.numpy as jnp
from jax import lax
import jax.experimental.pallas as pl
import jax.experimental.pallas.tpu as pltpu

S = 2048
D = 640
H = 32
DH = 20
F2 = 1536
FH = 768
NG = 4
GR = 160
GF = 320
GA = GR + 16
KS = (0, 128, 256, 384)
RR = ((0, 160), (0, 320), (160, 480), (320, 640), (480, 640))
TM = 256
NB = S // TM
EPS_LN = 1e-5
EPS_DEN = 1e-6
GELU_C = math.sqrt(2.0 / math.pi)
GELU_A = 0.044715

F32 = jnp.float32
BF16 = jnp.bfloat16


def _dot(a, b):
    return jnp.dot(a, b, preferred_element_type=F32)


def _dot_nt(a, b):
    return lax.dot_general(a, b, (((1,), (1,)), ((), ())), preferred_element_type=F32)


def _dot_tn(a, b):
    return lax.dot_general(a, b, (((0,), (0,)), ((), ())), preferred_element_type=F32)


def _ln(x):
    m = jnp.mean(x, axis=-1, keepdims=True)
    xc = x - m
    v = jnp.mean(xc * xc, axis=-1, keepdims=True)
    r = lax.rsqrt(v + EPS_LN)
    return xc * r, r


def _ln_bwd(dy, xn, r):
    a = jnp.mean(dy, axis=-1, keepdims=True)
    b = jnp.mean(dy * xn, axis=-1, keepdims=True)
    return r * (dy - a - xn * b)


def _iota(shape, dim):
    return lax.broadcasted_iota(jnp.int32, shape, dim)


def _row_map(r):
    g = ((r >= GR).astype(jnp.int32) + (r >= 2 * GR).astype(jnp.int32)
         + (r >= 3 * GR).astype(jnp.int32))
    rem = r - GR * g
    return rem >> 3, 8 * g + (rem & 7)


def _tile(r, n):
    return jnp.concatenate([r] * n, axis=1)


def _phi_t(pt):
    p4 = pt.reshape(NG, DH, 8, pt.shape[1])
    mx = jnp.max(p4, axis=1, keepdims=True)
    mn = jnp.min(p4, axis=1, keepdims=True)
    ep = jnp.exp(p4 - mx)
    en = jnp.exp(mn - p4)
    sp = jnp.sum(ep, axis=1, keepdims=True)
    sn = jnp.sum(en, axis=1, keepdims=True)
    return ep * (1.0 / sp), en * (1.0 / sn)


def _phi_bwd_t(php, phn, dphp, dphn):
    cp = jnp.sum(dphp * php, axis=1, keepdims=True)
    cn = jnp.sum(dphn * phn, axis=1, keepdims=True)
    return php * (dphp - cp) - phn * (dphn - cn)


def _gelu(u):
    t = jnp.tanh(u * (GELU_C + (GELU_C * GELU_A) * (u * u)))
    return u * (0.5 + 0.5 * t)


def _gelu_grad_parts(u):
    u2 = u * u
    t = jnp.tanh(u * (GELU_C + (GELU_C * GELU_A) * u2))
    hp = 0.5 + 0.5 * t
    da = hp + (u * (hp * (1.0 - hp))) * (2.0 * GELU_C + (6.0 * GELU_C * GELU_A) * u2)
    return hp, da


def _gelu_and_grad(u):
    hp, da = _gelu_grad_parts(u)
    return u * hp, da


def _kernel(
    x_hbm, wqkv_hbm, wphi_hbm, wo_hbm, win_hbm, wsp_hbm, bsp_hbm, wout_hbm, gout_hbm,
    out_hbm, dx_hbm, dwqkv_hbm, dwphi_hbm, dwo_hbm, dwin_hbm, dwsp_hbm, dbsp_hbm, dwout_hbm,
    sp_pq, sp_pk, sp_v, sp_o, sp_u, sp_g,
    xs_ref,
    hs_ref,
    rs_ref,
    gout_ref,
    dx_ref,
    pq_ref, pk_ref, v_ref, o_ref,
    u_ref,
    g_ref,
    z2_ref,
    dg_ref,
    wqkv_ref,
    wphi_ref,
    wphi2_ref,
    wo_ref,
    win_ref,
    wsp_ref,
    bsp_ref,
    wout_ref,
    wp_ref,
    phip_ref,
    pmt_ref,
    wop_ref,
    bcol_ref,
    dwp_ref,
    dwo_acc,
    dwin_acc,
    dwout_acc,
    kv_acc,
    kvm_ref,
    kvt_ref,
    dkvm_ref,
    dkvt_ref,
    rden_ref,
    r2_ref,
    dz_buf,
    ostage,
    wspstage,
    dbstage,
    dwphi_stage,
    sem_in, sem_spill, sem_rest, sem_out, sem_blk,
):
    def rows(i):
        if isinstance(i, int):
            return pl.ds(i * TM, TM)
        return pl.ds(pl.multiple_of(i * TM, TM), TM)

    wq_copies = [
        pltpu.make_async_copy(wqkv_hbm.at[:, t * D:(t + 1) * D], wqkv_ref.at[:, t * D:(t + 1) * D],
                              sem_in.at[9 + t])
        for t in range(3)
    ]
    pltpu.make_async_copy(wphi_hbm, wphi_ref, sem_in.at[2]).start()
    for c in wq_copies:
        c.start()
    in_copies = [
        pltpu.make_async_copy(x_hbm.at[0], xs_ref.at[0], sem_in.at[0]),
        None,
        None,
        pltpu.make_async_copy(wo_hbm, wo_ref, sem_in.at[3]),
        pltpu.make_async_copy(win_hbm, win_ref, sem_in.at[4]),
        pltpu.make_async_copy(bsp_hbm, bsp_ref, sem_in.at[5]),
        pltpu.make_async_copy(wsp_hbm, wsp_ref, sem_in.at[6]),
        pltpu.make_async_copy(wout_hbm, wout_ref, sem_in.at[7]),
        pltpu.make_async_copy(gout_hbm.at[0], gout_ref, sem_in.at[8]),
    ]
    for c in in_copies:
        if c is not None:
            c.start()

    def pmt_mat():
        f, head = _row_map(_iota((D, D), 0))
        return (_iota((D, D), 1) == head * DH + f).astype(BF16)

    def head_mask():
        c_dd = _iota((D, D), 1)
        _, head = _row_map(_iota((D, D), 0))
        hc = head * DH
        return jnp.logical_and(c_dd >= hc, c_dd < hc + DH)

    def et_mat():
        f, _ = _row_map(_iota((D, DH), 0))
        return (_iota((D, DH), 1) == f).astype(BF16)

    with jax.named_scope("prep"):
        dwp_ref[...] = jnp.zeros_like(dwp_ref)
        dwo_acc[...] = jnp.zeros_like(dwo_acc)
        dwin_acc[...] = jnp.zeros_like(dwin_acc)
        dwout_acc[...] = jnp.zeros_like(dwout_acc)
        pltpu.make_async_copy(wphi_hbm, wphi_ref, sem_in.at[2]).wait()
        for hh in range(H):
            wphi2_ref[hh * DH:(hh + 1) * DH, :] = wphi_ref[hh].astype(F32)
        phip_ref[...] = jnp.where(
            head_mask(), _dot_nt(et_mat(), wphi2_ref[...].astype(BF16)), 0.0).astype(BF16)
        pmt_ref[...] = pmt_mat()
        for t in range(3):
            wq_copies[t].wait()
            m_ref = phip_ref if t < 2 else pmt_ref
            for g in range(NG):
                wp_ref[t * D + g * GR:t * D + (g + 1) * GR, :] = _dot_nt(
                    m_ref[g * GR:(g + 1) * GR, KS[g]:KS[g] + 256],
                    wqkv_ref[:, t * D + KS[g]:t * D + KS[g] + 256]).astype(BF16)
        in_copies[3].wait()
        for g in range(NG):
            wop_ref[g * GR:(g + 1) * GR, :] = _dot(
                pmt_ref[g * GR:(g + 1) * GR, KS[g]:KS[g] + 256],
                wo_ref[KS[g]:KS[g] + 256, :]).astype(BF16)

    def kv_masks():
        r = _iota((384, 256), 0)
        c = _iota((384, 256), 1)
        return (r & 7) == (c & 7), c

    def a_fwd_finish(layer):
        same, c = kv_masks()
        keep = jnp.logical_and(same, c < GR + 8)
        for g in range(NG):
            m = kv_acc[g]
            zb = jnp.broadcast_to(m[:, GR:GR + 1], (384, 256))
            aug = jnp.where(keep, jnp.where(c < GR, m, zb), 0.0)
            kvm_ref[layer * NG + g] = aug[0:GF, 0:GA].astype(BF16)
            kvt_ref[layer * NG + g] = jnp.transpose(aug)[0:GA, 0:GF].astype(BF16)

    def a_bwd_finish():
        same, c = kv_masks()
        for g in range(NG):
            m = jnp.where(same, kv_acc[g], 0.0)
            dzc = jnp.sum(jnp.where(c >= GR, m, 0.0), axis=1, keepdims=True)
            mk = jnp.where(c < GR, m, 0.0)
            aug = jnp.where(c == GR, jnp.broadcast_to(dzc, (384, 256)), mk)
            dkvm_ref[g] = aug[0:GF, 0:GA].astype(BF16)
            dkvt_ref[g] = jnp.transpose(mk)[0:GR, 0:GF].astype(BF16)

    def ones_rows():
        return (_iota((GA - GR, TM), 0) == 0).astype(BF16)

    spill_bufs = [(pq_ref, sp_pq), (pk_ref, sp_pk), (v_ref, sp_v), (o_ref, sp_o),
                  (u_ref, sp_u), (g_ref, sp_g)]

    def spill_copy(k, i):
        src, dst = spill_bufs[k]
        idx = i if k < 4 else rows(i)
        return pltpu.make_async_copy(src.at[idx], dst.at[idx], sem_spill.at[k * NB + i])

    def spill_wait(k):
        for i in range(NB):
            spill_copy(k, i).wait()

    def restore_copy(k):
        dst, src = spill_bufs[k]
        return pltpu.make_async_copy(src, dst, sem_rest.at[k])

    def restore_u_copy(i):
        return pltpu.make_async_copy(sp_u.at[rows(i)], u_ref.at[rows(i)], sem_blk.at[i])

    def a_fwd1(layer, i):
        a_fwd1x(layer, i)
        a_fwd1y(i)

    def a_fwd1x(layer, i):
        x = xs_ref[0, rows(i), :].astype(F32)
        xn, r = _ln(x)
        h = xn.astype(BF16)
        hs_ref[2 * layer, rows(i), :] = h
        rs_ref[2 * layer, rows(i), :] = r
        pt = _dot_nt(wp_ref[...], h)
        pq = pt[0:D].astype(BF16)
        pk = pt[D:2 * D].astype(BF16)
        v = pt[2 * D:3 * D].astype(BF16)
        pq_ref[i] = pq
        pk_ref[i] = pk
        v_ref[i] = v
        if layer == 0:
            for k in range(3):
                spill_copy(k, i).start()

    def a_fwd1y(i):
        v = v_ref[i]
        kp, kn = _phi_t(pk_ref[i].astype(F32))
        phik = jnp.concatenate([kp, kn], axis=1).astype(BF16)
        for g in range(NG):
            va = jnp.concatenate([v[g * GR:(g + 1) * GR], ones_rows()], axis=0)
            kv_acc[g, 0:GF, 0:GA] += _dot_nt(phik[g].reshape(GF, TM), va)

    def a_fwd2(layer, i):
        x = xs_ref[0, rows(i), :].astype(F32)
        qp, qn = _phi_t(pq_ref[i].astype(F32))
        phiq = jnp.concatenate([qp, qn], axis=1).astype(BF16)
        os_, rds = [], []
        for g in range(NG):
            res = _dot(kvt_ref[layer * NG + g], phiq[g].reshape(GF, TM))
            rd = 1.0 / (res[GR:GR + 8] + EPS_DEN)
            rds.append(rd)
            os_.append(res[0:GR].reshape(DH, 8, TM) * rd[None])
        rden_ref[layer, i] = jnp.concatenate(rds, axis=0)
        o = jnp.concatenate(os_, axis=0).reshape(D, TM).astype(BF16)
        o_ref[i] = o
        if layer == 0:
            spill_copy(3, i).start()
        x1 = (x + _dot_tn(o, wop_ref[...])).astype(BF16)
        xs_ref[1, rows(i), :] = x1

    def b_fwd1(layer, i, x1):
        xn, r = _ln(x1.astype(F32))
        h = xn.astype(BF16)
        hs_ref[2 * layer + 1, rows(i), :] = h
        rs_ref[2 * layer + 1, rows(i), :] = r
        u = _dot(h, win_ref[...]).astype(BF16)
        u_ref[rows(i), :] = u
        if layer == 0:
            spill_copy(4, i).start()
        a2 = _gelu(u[:, FH:F2].astype(F32))
        z2, r2 = _ln(a2)
        z2_ref[rows(i), layer * FH:(layer + 1) * FH] = z2.astype(BF16)
        r2_ref[layer, rows(i), :] = r2

    def b_fwd2(layer, i, gl=None):
        x1 = xs_ref[1, rows(i), :].astype(F32)
        g = _dot(wsp_ref[rows(i), :], z2_ref[:, layer * FH:(layer + 1) * FH])
        g = (g + _tile(bcol_ref[rows(i), :], FH // 128)).astype(BF16)
        g_ref[rows(i), :] = g
        if layer == 0:
            spill_copy(5, i).start()
        z1 = _gelu(u_ref[rows(i), 0:FH].astype(F32)) if gl is None else gl[0]
        y = (z1 * g.astype(F32)).astype(BF16)
        x2 = (x1 + _dot(y, wout_ref[...])).astype(BF16)
        return x2

    def b_bwd1(layer, i, dy, gl=None):
        dyb = dy.astype(BF16)
        g = g_ref[rows(i), :].astype(F32)
        z1, dgelu1 = _gelu_and_grad(u_ref[rows(i), 0:FH].astype(F32)) if gl is None else gl
        y = (z1 * g).astype(BF16)
        dzg = _dot_nt(dyb, wout_ref[...])
        dwout_acc[...] += _dot_tn(y, dyb)
        dg = (dzg * z1).astype(BF16)
        dg_ref[rows(i), layer * FH:(layer + 1) * FH] = dg
        du1 = (dzg * g * dgelu1).astype(BF16)
        h = hs_ref[2 * layer + 1, rows(i), :]
        gout_ref[rows(i), :] = _dot_nt(du1, win_ref[:, 0:FH]).astype(BF16)
        dwin_acc[:, 0:FH] += _dot_tn(h, du1)

    def b_bwd2x(layer, i):
        return _dot_tn(wsp_ref[:, rows(i)], dg_ref[:, layer * FH:(layer + 1) * FH])

    def b_bwd2(layer, i, dxp, dz2):
        _, dgelu2 = _gelu_grad_parts(u_ref[rows(i), FH:F2].astype(F32))
        z2n = z2_ref[rows(i), layer * FH:(layer + 1) * FH].astype(F32)
        du2 = (_ln_bwd(dz2, z2n, r2_ref[layer, rows(i), :]) * dgelu2).astype(BF16)
        h = hs_ref[2 * layer + 1, rows(i), :]
        dh = _dot_nt(du2, win_ref[:, FH:F2]) + gout_ref[rows(i), :].astype(F32)
        dwin_acc[:, FH:F2] += _dot_tn(h, du2)
        return dxp + _ln_bwd(dh, h.astype(F32), rs_ref[2 * layer + 1, rows(i), :])

    def a_bwd1(layer, i, dy):
        dyb = dy.astype(BF16)
        ob = o_ref[i]
        do = _dot_nt(wop_ref[...], dyb).reshape(NG, DH, 8, TM)
        dwo_acc[...] += _dot(ob, dyb)
        qp, qn = _phi_t(pq_ref[i].astype(F32))
        phiq = jnp.concatenate([qp, qn], axis=1).astype(BF16)
        rden = rden_ref[layer, i].reshape(NG, 1, 8, TM)
        dden = -jnp.sum(do * ob.astype(F32).reshape(NG, DH, 8, TM), axis=1, keepdims=True) * rden
        dna = jnp.concatenate([do * rden, dden, jnp.zeros_like(dden)], axis=1).astype(BF16)
        dphi = []
        for g in range(NG):
            dn = dna[g].reshape(GA, TM)
            dphi.append(_dot(kvm_ref[layer * NG + g], dn))
            kv_acc[g, 0:GF, 0:GA] += _dot_nt(phiq[g].reshape(GF, TM), dn)
        dphi = jnp.concatenate(dphi, axis=0).reshape(NG, 2 * DH, 8, TM)
        dpq = _phi_bwd_t(qp, qn, dphi[:, 0:DH], dphi[:, DH:2 * DH]).reshape(D, TM).astype(BF16)
        h = hs_ref[2 * layer, rows(i), :]
        gout_ref[rows(i), :] = _dot_tn(dpq, wp_ref[0:D, :]).astype(BF16)
        dwp_ref[0:D, :] += _dot(dpq, h)

    def a_bwd2(layer, i, dxp):
        v = v_ref[i]
        kp, kn = _phi_t(pk_ref[i].astype(F32))
        phik = jnp.concatenate([kp, kn], axis=1).astype(BF16)
        dphi, dvs = [], []
        for g in range(NG):
            va = jnp.concatenate([v[g * GR:(g + 1) * GR], ones_rows()], axis=0)
            dphi.append(_dot(dkvm_ref[g], va))
            dvs.append(_dot(dkvt_ref[g], phik[g].reshape(GF, TM)))
        dphi = jnp.concatenate(dphi, axis=0).reshape(NG, 2 * DH, 8, TM)
        dpk = _phi_bwd_t(kp, kn, dphi[:, 0:DH], dphi[:, DH:2 * DH]).reshape(D, TM)
        dkv = jnp.concatenate([dpk] + dvs, axis=0).astype(BF16)
        h = hs_ref[2 * layer, rows(i), :]
        dh = _dot_tn(dkv, wp_ref[D:3 * D, :]) + gout_ref[rows(i), :].astype(F32)
        dwp_ref[D:3 * D, :] += _dot(dkv, h)
        return dxp + _ln_bwd(dh, h.astype(F32), rs_ref[2 * layer, rows(i), :])

    def loop(body, name="loop", unroll=1):
        def b(i, c):
            for k in range(unroll):
                body(i * unroll + k)
            return c
        with jax.named_scope(name):
            lax.fori_loop(0, NB // unroll, b, 0)

    def stage_out(i, val, dst_hbm, stage, semoff):
        slot = i % 2

        @pl.when(i >= 2)
        def _():
            pltpu.make_async_copy(stage.at[slot], dst_hbm.at[rows(i - 2)],
                                  sem_blk.at[semoff + slot]).wait()
        stage[slot] = val
        pltpu.make_async_copy(stage.at[slot], dst_hbm.at[rows(i)], sem_blk.at[semoff + slot]).start()

    def stage_drain(dst_hbm, stage, semoff):
        for i in (NB - 2, NB - 1):
            slot = i % 2
            pltpu.make_async_copy(stage.at[slot], dst_hbm.at[rows(i)],
                                  sem_blk.at[semoff + slot]).wait()

    with jax.named_scope("pre1"):
        in_copies[0].wait()
        kv_acc[...] = jnp.zeros_like(kv_acc)
    with jax.named_scope("P1"):
        a_fwd1x(0, 0)

        def p1(i, c):
            a_fwd1y(i)
            a_fwd1x(0, i + 1)
            return c
        lax.fori_loop(0, NB - 1, p1, 0)
        a_fwd1y(NB - 1)

    with jax.named_scope("pre2"):
        a_fwd_finish(0)
        in_copies[4].wait()
        in_copies[5].wait()
        bcol_ref[...] = jnp.transpose(
            jnp.broadcast_to(bsp_ref[...].astype(F32), (128, S)))

    def p2(layer, name):
        with jax.named_scope(name):
            a_fwd2(layer, 0)

            def body(i, c):
                x1 = xs_ref[1, rows(i), :]
                a_fwd2(layer, i + 1)
                b_fwd1(layer, i, x1)
                return c
            lax.fori_loop(0, NB - 1, body, 0)
            b_fwd1(layer, NB - 1, xs_ref[1, rows(NB - 1), :])
    p2(0, "P2")

    with jax.named_scope("pre3"):
        in_copies[6].wait()
        in_copies[7].wait()
        for k in range(3):
            spill_wait(k)
        kv_acc[...] = jnp.zeros_like(kv_acc)

    with jax.named_scope("P3"):
        xs_ref[0, rows(0), :] = b_fwd2(0, 0)
        a_fwd1x(1, 0)

        def p3(i, c):
            a_fwd1y(i)
            xs_ref[0, rows(i + 1), :] = b_fwd2(0, i + 1)
            a_fwd1x(1, i + 1)
            return c
        lax.fori_loop(0, NB - 1, p3, 0)
        a_fwd1y(NB - 1)

    with jax.named_scope("pre4"):
        a_fwd_finish(1)
        spill_wait(3)
        spill_wait(4)
    p2(1, "P4")

    with jax.named_scope("pre5"):
        spill_wait(5)
        in_copies[8].wait()

    def p5(i):
        gl = _gelu_and_grad(u_ref[rows(i), 0:FH].astype(F32))
        x4 = b_fwd2(1, i, gl)
        stage_out(i, x4, out_hbm.at[0], ostage, NB)
        dy = gout_ref[rows(i), :].astype(F32)
        dx_ref[rows(i), :] = dy
        b_bwd1(1, i, dy, gl)
    loop(p5, "P5", 2)

    with jax.named_scope("pre6"):
        stage_drain(out_hbm.at[0], ostage, NB)
        restore_copy(5).start()
        kv_acc[...] = jnp.zeros_like(kv_acc)

    def p6(layer, name):
        with jax.named_scope(name):
            dz_buf[0] = b_bwd2x(layer, 0)

            def step(i, slot, last):
                dz2 = dz_buf[slot]
                if not last:
                    dzn = b_bwd2x(layer, i + 1)
                dx3 = b_bwd2(layer, i, dx_ref[rows(i), :], dz2)
                dx_ref[rows(i), :] = dx3
                if layer == 1:
                    restore_u_copy(i).start()
                a_bwd1(layer, i, dx3)
                if not last:
                    dz_buf[1 - slot] = dzn

            def body(i, c):
                step(i, i % 2, False)
                return c
            lax.fori_loop(0, NB - 1, body, 0)
            step(NB - 1, (NB - 1) % 2, True)
    p6(1, "P6")

    with jax.named_scope("pre7"):
        a_bwd_finish()
        restore_copy(0).start()
        restore_copy(3).start()
        restore_copy(5).wait()
        for i in range(NB):
            restore_u_copy(i).wait()

    def p7(i):
        dx2 = a_bwd2(1, i, dx_ref[rows(i), :])
        dx_ref[rows(i), :] = dx2
        b_bwd1(0, i, dx2)
    loop(p7, "P7")

    db_copy = pltpu.make_async_copy(dbstage, dbsp_hbm, sem_out.at[0])
    with jax.named_scope("pre8"):
        restore_copy(1).start()
        restore_copy(2).start()
        restore_copy(0).wait()
        restore_copy(3).wait()
        kv_acc[...] = jnp.zeros_like(kv_acc)
    p6(0, "P8")

    def dwqkv_copy(t):
        return pltpu.make_async_copy(wqkv_ref.at[:, t * D:(t + 1) * D],
                                     dwqkv_hbm.at[:, t * D:(t + 1) * D], sem_out.at[6 + t])

    def unfold(t):
        m_ref = phip_ref if t < 2 else pmt_ref
        for j in range(5):
            r0, r1 = RR[j]
            wqkv_ref[:, t * D + 128 * j:t * D + 128 * (j + 1)] = _dot_tn(
                wp_ref[t * D + r0:t * D + r1, :],
                m_ref[r0:r1, 128 * j:128 * (j + 1)]).astype(BF16)
        dwqkv_copy(t).start()

    dwin_copy = pltpu.make_async_copy(win_ref, dwin_hbm, sem_out.at[1])
    dwout_copy = pltpu.make_async_copy(wout_ref, dwout_hbm, sem_out.at[2])
    dwo_copy = pltpu.make_async_copy(wo_ref, dwo_hbm, sem_out.at[3])
    with jax.named_scope("pre9"):
        a_bwd_finish()
        win_ref[...] = dwin_acc[...].astype(BF16)
        dwin_copy.start()
        wout_ref[...] = dwout_acc[...].astype(BF16)
        dwout_copy.start()
        wop_ref[...] = dwo_acc[...].astype(BF16)
        for j in range(5):
            r0, r1 = RR[j]
            wo_ref[128 * j:128 * (j + 1), :] = _dot_tn(
                pmt_ref[r0:r1, 128 * j:128 * (j + 1)], wop_ref[r0:r1, :]).astype(BF16)
        dwo_copy.start()
        wp_ref[0:D, :] = dwp_ref[0:D, :].astype(BF16)
        dwo_acc[...] = jnp.zeros_like(dwo_acc)
        for g in range(NG):
            dwo_acc[g * GR:(g + 1) * GR, KS[g]:KS[g] + 256] = _dot(
                wp_ref[g * GR:(g + 1) * GR, :], wqkv_ref[:, KS[g]:KS[g] + 256])
        unfold(0)
        restore_copy(1).wait()
        restore_copy(2).wait()

    def p9(i):
        dgb = dg_ref[rows(i), :]
        dwsp = _dot_nt(dgb, z2_ref[...]).astype(BF16)
        db = _dot_nt(jnp.ones((8, 2 * FH), BF16), dgb)
        dx0 = a_bwd2(0, i, dx_ref[rows(i), :])
        stage_out(i, dwsp, dwsp_hbm, wspstage, NB + 2)
        dbstage[:, pl.ds(pl.multiple_of(i * TM, TM), TM)] = db[0:1, :].astype(BF16)
        stage_out(i, dx0.astype(BF16), dx_hbm.at[0], ostage, NB)
    loop(p9, "P9")

    dwphi_copy = pltpu.make_async_copy(dwphi_stage, dwphi_hbm, sem_out.at[5])
    with jax.named_scope("final"):
        db_copy.start()
        wp_ref[D:3 * D, :] = dwp_ref[D:3 * D, :].astype(BF16)
        unfold(2)
        for g in range(NG):
            dwo_acc[g * GR:(g + 1) * GR, KS[g]:KS[g] + 256] += _dot(
                wp_ref[D + g * GR:D + (g + 1) * GR, :], wqkv_ref[:, D + KS[g]:D + KS[g] + 256])
        unfold(1)
        mm = jnp.where(head_mask(), dwo_acc[...], 0.0)
        mhi = mm.astype(BF16)
        mlo = (mm - mhi.astype(F32)).astype(BF16)
        wphi2_ref[...] = _dot_tn(mhi, et_mat()) + _dot_tn(mlo, et_mat())
        for hh in range(H):
            dwphi_stage[hh] = wphi2_ref[hh * DH:(hh + 1) * DH, :].astype(BF16)
        dwphi_copy.start()

    with jax.named_scope("drain"):
        stage_drain(dwsp_hbm, wspstage, NB + 2)
        stage_drain(dx_hbm.at[0], ostage, NB)
        db_copy.wait()
        dwin_copy.wait()
        dwout_copy.wait()
        dwo_copy.wait()
        for t in range(3):
            dwqkv_copy(t).wait()
        dwphi_copy.wait()


@jax.jit
def pallas_interleave_layers__linear_kernel_hedgehog__mixer_gmlp__prompt_kernel(
    A_x: jax.Array,
    A_wqkv: jax.Array,
    A_w_phi: jax.Array,
    A_wo: jax.Array,
    B_x: jax.Array,
    B_w_in: jax.Array,
    B_w_sp: jax.Array,
    B_b_sp: jax.Array,
    B_w_out: jax.Array,
    grad_out: jax.Array,
):
    del B_x
    bsp2d = B_b_sp.reshape(1, S)

    any_spec = pl.BlockSpec(memory_space=pl.ANY)
    out_shape = (
        jax.ShapeDtypeStruct((1, S, D), BF16),
        jax.ShapeDtypeStruct((1, S, D), BF16),
        jax.ShapeDtypeStruct((D, 3 * D), BF16),
        jax.ShapeDtypeStruct((H, DH, DH), BF16),
        jax.ShapeDtypeStruct((D, D), BF16),
        jax.ShapeDtypeStruct((D, F2), BF16),
        jax.ShapeDtypeStruct((S, S), BF16),
        jax.ShapeDtypeStruct((1, S), BF16),
        jax.ShapeDtypeStruct((FH, D), BF16),
        jax.ShapeDtypeStruct((NB, D, TM), BF16),
        jax.ShapeDtypeStruct((NB, D, TM), BF16),
        jax.ShapeDtypeStruct((NB, D, TM), BF16),
        jax.ShapeDtypeStruct((NB, D, TM), BF16),
        jax.ShapeDtypeStruct((S, F2), BF16),
        jax.ShapeDtypeStruct((S, FH), BF16),
    )
    scratch_shapes = [
        pltpu.VMEM((2, S, D), BF16),
        pltpu.VMEM((4, S, D), BF16),
        pltpu.VMEM((4, S, 1), F32),
        pltpu.VMEM((S, D), BF16),
        pltpu.VMEM((S, D), F32),
        pltpu.VMEM((NB, D, TM), BF16),
        pltpu.VMEM((NB, D, TM), BF16),
        pltpu.VMEM((NB, D, TM), BF16),
        pltpu.VMEM((NB, D, TM), BF16),
        pltpu.VMEM((S, F2), BF16),
        pltpu.VMEM((S, FH), BF16),
        pltpu.VMEM((S, 2 * FH), BF16),
        pltpu.VMEM((S, 2 * FH), BF16),
        pltpu.VMEM((D, 3 * D), BF16),
        pltpu.VMEM((H, DH, DH), BF16),
        pltpu.VMEM((D, DH), F32),
        pltpu.VMEM((D, D), BF16),
        pltpu.VMEM((D, F2), BF16),
        pltpu.VMEM((S, S), BF16),
        pltpu.VMEM((1, S), BF16),
        pltpu.VMEM((FH, D), BF16),
        pltpu.VMEM((3 * D, D), BF16),
        pltpu.VMEM((D, D), BF16),
        pltpu.VMEM((D, D), BF16),
        pltpu.VMEM((D, D), BF16),
        pltpu.VMEM((S, 128), F32),
        pltpu.VMEM((3 * D, D), F32),
        pltpu.VMEM((D, D), F32),
        pltpu.VMEM((D, F2), F32),
        pltpu.VMEM((FH, D), F32),
        pltpu.VMEM((NG, 384, 256), F32),
        pltpu.VMEM((2 * NG, GF, GA), BF16),
        pltpu.VMEM((2 * NG, GA, GF), BF16),
        pltpu.VMEM((NG, GF, GA), BF16),
        pltpu.VMEM((NG, GR, GF), BF16),
        pltpu.VMEM((2, NB, H, TM), F32),
        pltpu.VMEM((2, S, 1), F32),
        pltpu.VMEM((2, TM, FH), F32),
        pltpu.VMEM((2, TM, D), BF16),
        pltpu.VMEM((2, TM, S), BF16),
        pltpu.VMEM((1, S), BF16),
        pltpu.VMEM((H, DH, DH), BF16),
        pltpu.SemaphoreType.DMA((12,)),
        pltpu.SemaphoreType.DMA((6 * NB,)),
        pltpu.SemaphoreType.DMA((6,)),
        pltpu.SemaphoreType.DMA((9,)),
        pltpu.SemaphoreType.DMA((NB + 4,)),
    ]
    outs = pl.pallas_call(
        _kernel,
        out_shape=out_shape,
        in_specs=[any_spec] * 9,
        out_specs=tuple([any_spec] * len(out_shape)),
        scratch_shapes=scratch_shapes,
        compiler_params=pltpu.CompilerParams(
            vmem_limit_bytes=125 * 1024 * 1024,
        ),
    )(A_x, A_wqkv, A_w_phi, A_wo, B_w_in, B_w_sp, bsp2d, B_w_out, grad_out)
    out, dx0, dwqkv, dwphi, dwo, dwin, dwsp, dbsp, dwout = outs[:9]
    return (out, dx0, dwqkv, dwphi, dwo, dwin, dwsp,
            dbsp.reshape(S), dwout)
```

```python
import math

import jax
import jax.numpy as jnp
from jax import lax
import jax.experimental.pallas as pl
import jax.experimental.pallas.tpu as pltpu

S = 2048
D = 640
H = 32
DH = 20
F2 = 1536
FH = 768
NG = 8
GR = 80
GF = 160
GA = GR + 16
NV = DH // 2
SG = 4
SR = 160
KS = (0, 128, 256, 384)
RR = ((0, 160), (0, 320), (160, 480), (320, 640), (480, 640))
TM = 256
NB = S // TM
EPS_LN = 1e-5
EPS_DEN = 1e-6
GELU_C = math.sqrt(2.0 / math.pi)
GELU_A = 0.044715

F32 = jnp.float32
BF16 = jnp.bfloat16


def _dot(a, b):
    return jnp.dot(a, b, preferred_element_type=F32)


def _dot_nt(a, b):
    return lax.dot_general(a, b, (((1,), (1,)), ((), ())), preferred_element_type=F32)


def _dot_tn(a, b):
    return lax.dot_general(a, b, (((0,), (0,)), ((), ())), preferred_element_type=F32)


def _ln(x):
    m = jnp.mean(x, axis=-1, keepdims=True)
    xc = x - m
    v = jnp.mean(xc * xc, axis=-1, keepdims=True)
    r = lax.rsqrt(v + EPS_LN)
    return xc * r, r


def _ln_bwd(dy, xn, r):
    a = jnp.mean(dy, axis=-1, keepdims=True)
    b = jnp.mean(dy * xn, axis=-1, keepdims=True)
    return r * (dy - a - xn * b)


def _iota(shape, dim):
    return lax.broadcasted_iota(jnp.int32, shape, dim)


def _row_map(r):
    g = (r * 205) >> 14
    rem = r - GR * g
    return rem >> 2, 4 * g + (rem & 3)


def _tile(r, n):
    return jnp.concatenate([r] * n, axis=1)


def _hred(x, red, op):
    r = red(x, axis=1)
    r = op(r, pltpu.roll(r, 4, 1))
    return r[:, None]


def _phi_t(pt):
    p4 = pt.reshape(NG, NV, 8, pt.shape[1])
    mx = _hred(p4, jnp.max, jnp.maximum)
    mn = _hred(p4, jnp.min, jnp.minimum)
    ep = jnp.exp(p4 - mx)
    en = jnp.exp(mn - p4)
    sp = _hred(ep, jnp.sum, jnp.add)
    sn = _hred(en, jnp.sum, jnp.add)
    return ep * (1.0 / sp), en * (1.0 / sn)


def _phi_bwd_t(php, phn, dphp, dphn):
    cp = _hred(dphp * php, jnp.sum, jnp.add)
    cn = _hred(dphn * phn, jnp.sum, jnp.add)
    return php * (dphp - cp) - phn * (dphn - cn)


def _gelu(u):
    t = jnp.tanh(u * (GELU_C + (GELU_C * GELU_A) * (u * u)))
    return u * (0.5 + 0.5 * t)


def _gelu_grad_parts(u):
    u2 = u * u
    t = jnp.tanh(u * (GELU_C + (GELU_C * GELU_A) * u2))
    hp = 0.5 + 0.5 * t
    da = hp + (u * (hp * (1.0 - hp))) * (2.0 * GELU_C + (6.0 * GELU_C * GELU_A) * u2)
    return hp, da


def _gelu_and_grad(u):
    hp, da = _gelu_grad_parts(u)
    return u * hp, da


def _kernel(
    x_hbm, wqkv_hbm, wphi_hbm, wo_hbm, win_hbm, wsp_hbm, bsp_hbm, wout_hbm, gout_hbm,
    out_hbm, dx_hbm, dwqkv_hbm, dwphi_hbm, dwo_hbm, dwin_hbm, dwsp_hbm, dbsp_hbm, dwout_hbm,
    sp_pq, sp_pk, sp_v, sp_o, sp_u, sp_g,
    xs_ref,
    hs_ref,
    rs_ref,
    gout_ref,
    dx_ref,
    pq_ref, pk_ref, v_ref, o_ref,
    u_ref,
    g_ref,
    z2_ref,
    dg_ref,
    wqkv_ref,
    wphi_ref,
    wphi2_ref,
    wo_ref,
    win_ref,
    wsp_ref,
    bsp_ref,
    wout_ref,
    wp_ref,
    phip_ref,
    pmt_ref,
    wop_ref,
    bcol_ref,
    dwp_ref,
    dwo_acc,
    dwin_acc,
    dwout_acc,
    kv_acc,
    kvm_ref,
    kvt_ref,
    dkvm_ref,
    dkvt_ref,
    rden_ref,
    r2_ref,
    dz_buf,
    ostage,
    wspstage,
    dbstage,
    dwphi_stage,
    sem_in, sem_spill, sem_rest, sem_out, sem_blk,
):
    def rows(i):
        if isinstance(i, int):
            return pl.ds(i * TM, TM)
        return pl.ds(pl.multiple_of(i * TM, TM), TM)

    wq_copies = [
        pltpu.make_async_copy(wqkv_hbm.at[:, t * D:(t + 1) * D], wqkv_ref.at[:, t * D:(t + 1) * D],
                              sem_in.at[9 + t])
        for t in range(3)
    ]
    pltpu.make_async_copy(wphi_hbm, wphi_ref, sem_in.at[2]).start()
    for c in wq_copies:
        c.start()
    in_copies = [
        pltpu.make_async_copy(x_hbm.at[0], xs_ref.at[0], sem_in.at[0]),
        None,
        None,
        pltpu.make_async_copy(wo_hbm, wo_ref, sem_in.at[3]),
        pltpu.make_async_copy(win_hbm, win_ref, sem_in.at[4]),
        pltpu.make_async_copy(bsp_hbm, bsp_ref, sem_in.at[5]),
        pltpu.make_async_copy(wsp_hbm, wsp_ref, sem_in.at[6]),
        pltpu.make_async_copy(wout_hbm, wout_ref, sem_in.at[7]),
        pltpu.make_async_copy(gout_hbm.at[0], gout_ref, sem_in.at[8]),
    ]
    for c in in_copies:
        if c is not None:
            c.start()

    def pmt_mat():
        f, head = _row_map(_iota((D, D), 0))
        return (_iota((D, D), 1) == head * DH + f).astype(BF16)

    def head_mask():
        c_dd = _iota((D, D), 1)
        _, head = _row_map(_iota((D, D), 0))
        hc = head * DH
        return jnp.logical_and(c_dd >= hc, c_dd < hc + DH)

    def et_mat():
        f, _ = _row_map(_iota((D, DH), 0))
        return (_iota((D, DH), 1) == f).astype(BF16)

    with jax.named_scope("prep"):
        dwp_ref[...] = jnp.zeros_like(dwp_ref)
        dwo_acc[...] = jnp.zeros_like(dwo_acc)
        dwin_acc[...] = jnp.zeros_like(dwin_acc)
        dwout_acc[...] = jnp.zeros_like(dwout_acc)
        pltpu.make_async_copy(wphi_hbm, wphi_ref, sem_in.at[2]).wait()
        for hh in range(H):
            wphi2_ref[hh * DH:(hh + 1) * DH, :] = wphi_ref[hh].astype(F32)
        phip_ref[...] = jnp.where(
            head_mask(), _dot_nt(et_mat(), wphi2_ref[...].astype(BF16)), 0.0).astype(BF16)
        pmt_ref[...] = pmt_mat()
        for t in range(3):
            wq_copies[t].wait()
            m_ref = phip_ref if t < 2 else pmt_ref
            for g in range(SG):
                wp_ref[t * D + g * SR:t * D + (g + 1) * SR, :] = _dot_nt(
                    m_ref[g * SR:(g + 1) * SR, KS[g]:KS[g] + 256],
                    wqkv_ref[:, t * D + KS[g]:t * D + KS[g] + 256]).astype(BF16)
        in_copies[5].wait()
        bcol_ref[...] = jnp.transpose(
            jnp.broadcast_to(bsp_ref[...].astype(F32), (128, S)))
        in_copies[3].wait()
        for g in range(SG):
            wop_ref[g * SR:(g + 1) * SR, :] = _dot(
                pmt_ref[g * SR:(g + 1) * SR, KS[g]:KS[g] + 256],
                wo_ref[KS[g]:KS[g] + 256, :]).astype(BF16)

    def kv_masks():
        r = _iota((256, 128), 0)
        c = _iota((256, 128), 1)
        return (r & 3) == (c & 3), c

    def a_fwd_finish(layer):
        same, c = kv_masks()
        keep = jnp.logical_and(same, c < GR + 8)
        for g in range(NG):
            m = kv_acc[g]
            zb = jnp.broadcast_to(m[:, GR:GR + 1], (256, 128))
            aug = jnp.where(keep, jnp.where(c < GR, m, zb), 0.0)
            kvm_ref[layer * NG + g] = aug[0:GF, 0:GA].astype(BF16)
            kvt_ref[layer * NG + g] = jnp.transpose(aug)[0:GA, 0:GF].astype(BF16)

    def a_bwd_finish():
        same, c = kv_masks()
        for g in range(NG):
            m = jnp.where(same, kv_acc[g], 0.0)
            dzc = jnp.sum(jnp.where(c >= GR, m, 0.0), axis=1, keepdims=True)
            mk = jnp.where(c < GR, m, 0.0)
            aug = jnp.where(c == GR, jnp.broadcast_to(dzc, (256, 128)), mk)
            dkvm_ref[g] = aug[0:GF, 0:GA].astype(BF16)
            dkvt_ref[g] = jnp.transpose(mk)[0:GR, 0:GF].astype(BF16)

    def ones_rows():
        return (_iota((GA - GR, TM), 0) == 0).astype(BF16)

    spill_bufs = [(pq_ref, sp_pq), (pk_ref, sp_pk), (v_ref, sp_v), (o_ref, sp_o),
                  (u_ref, sp_u), (g_ref, sp_g)]

    def spill_copy(k, i):
        src, dst = spill_bufs[k]
        idx = i if k < 4 else rows(i)
        return pltpu.make_async_copy(src.at[idx], dst.at[idx], sem_spill.at[k * NB + i])

    def spill_wait(k):
        for i in range(NB):
            spill_copy(k, i).wait()

    def restore_copy(k):
        dst, src = spill_bufs[k]
        return pltpu.make_async_copy(src, dst, sem_rest.at[k])

    def restore_u_copy(i):
        return pltpu.make_async_copy(sp_u.at[rows(i)], u_ref.at[rows(i)], sem_blk.at[i])

    def a_fwd1(layer, i):
        a_fwd1x(layer, i)
        a_fwd1y(i)

    def a_fwd1x(layer, i):
        x = xs_ref[0, rows(i), :].astype(F32)
        xn, r = _ln(x)
        h = xn.astype(BF16)
        hs_ref[2 * layer, rows(i), :] = h
        rs_ref[2 * layer, rows(i), :] = r
        pt = _dot_nt(wp_ref[...], h)
        pq = pt[0:D].astype(BF16)
        pk = pt[D:2 * D].astype(BF16)
        v = pt[2 * D:3 * D].astype(BF16)
        pq_ref[i] = pq
        pk_ref[i] = pk
        v_ref[i] = v
        if layer == 0:
            for k in range(3):
                spill_copy(k, i).start()

    def a_fwd1y(i):
        v = v_ref[i]
        kp, kn = _phi_t(pk_ref[i].astype(F32))
        phik = jnp.concatenate([kp, kn], axis=1).astype(BF16)
        for g in range(NG):
            va = jnp.concatenate([v[g * GR:(g + 1) * GR], ones_rows()], axis=0)
            kv_acc[g, 0:GF, 0:GA] += _dot_nt(phik[g].reshape(GF, TM), va)

    def a_fwd2(layer, i):
        x = xs_ref[0, rows(i), :].astype(F32)
        qp, qn = _phi_t(pq_ref[i].astype(F32))
        phiq = jnp.concatenate([qp, qn], axis=1).astype(BF16)
        os_, rds = [], []
        for g in range(NG):
            res = _dot(kvt_ref[layer * NG + g], phiq[g].reshape(GF, TM))
            rd = 1.0 / (res[GR:GR + 8] + EPS_DEN)
            rds.append(rd)
            os_.append(res[0:GR].reshape(NV, 8, TM) * rd[None])
        rden_ref[layer, i] = jnp.concatenate(rds, axis=0)
        o = jnp.concatenate(os_, axis=0).reshape(D, TM).astype(BF16)
        o_ref[i] = o
        if layer == 0:
            spill_copy(3, i).start()
        x1 = (x + _dot_tn(o, wop_ref[...])).astype(BF16)
        xs_ref[1, rows(i), :] = x1

    def b_fwd1(layer, i, x1):
        xn, r = _ln(x1.astype(F32))
        h = xn.astype(BF16)
        hs_ref[2 * layer + 1, rows(i), :] = h
        rs_ref[2 * layer + 1, rows(i), :] = r
        u = _dot(h, win_ref[...]).astype(BF16)
        u_ref[rows(i), :] = u
        if layer == 0:
            spill_copy(4, i).start()
        a2 = _gelu(u[:, FH:F2].astype(F32))
        z2, r2 = _ln(a2)
        z2_ref[rows(i), layer * FH:(layer + 1) * FH] = z2.astype(BF16)
        r2_ref[layer, rows(i), :] = r2

    def b_fwd2(layer, i, gl=None):
        x1 = xs_ref[1, rows(i), :].astype(F32)
        g = _dot(wsp_ref[rows(i), :], z2_ref[:, layer * FH:(layer + 1) * FH])
        g = (g + _tile(bcol_ref[rows(i), :], FH // 128)).astype(BF16)
        g_ref[rows(i), :] = g
        if layer == 0:
            spill_copy(5, i).start()
        z1 = _gelu(u_ref[rows(i), 0:FH].astype(F32)) if gl is None else gl[0]
        y = (z1 * g.astype(F32)).astype(BF16)
        x2 = (x1 + _dot(y, wout_ref[...])).astype(BF16)
        return x2

    def b_bwd1(layer, i, dy, gl=None):
        dyb = dy.astype(BF16)
        g = g_ref[rows(i), :].astype(F32)
        z1, dgelu1 = _gelu_and_grad(u_ref[rows(i), 0:FH].astype(F32)) if gl is None else gl
        y = (z1 * g).astype(BF16)
        dzg = _dot_nt(dyb, wout_ref[...])
        dwout_acc[...] += _dot_tn(y, dyb)
        dg = (dzg * z1).astype(BF16)
        dg_ref[rows(i), layer * FH:(layer + 1) * FH] = dg
        du1 = (dzg * g * dgelu1).astype(BF16)
        h = hs_ref[2 * layer + 1, rows(i), :]
        gout_ref[rows(i), :] = _dot_nt(du1, win_ref[:, 0:FH]).astype(BF16)
        dwin_acc[:, 0:FH] += _dot_tn(h, du1)

    def b_bwd2x(layer, i):
        return _dot_tn(wsp_ref[:, rows(i)], dg_ref[:, layer * FH:(layer + 1) * FH])

    def b_bwd2(layer, i, dxp, dz2):
        _, dgelu2 = _gelu_grad_parts(u_ref[rows(i), FH:F2].astype(F32))
        z2n = z2_ref[rows(i), layer * FH:(layer + 1) * FH].astype(F32)
        du2 = (_ln_bwd(dz2, z2n, r2_ref[layer, rows(i), :]) * dgelu2).astype(BF16)
        h = hs_ref[2 * layer + 1, rows(i), :]
        dh = _dot_nt(du2, win_ref[:, FH:F2]) + gout_ref[rows(i), :].astype(F32)
        dwin_acc[:, FH:F2] += _dot_tn(h, du2)
        return dxp + _ln_bwd(dh, h.astype(F32), rs_ref[2 * layer + 1, rows(i), :])

    def a_bwd1(layer, i, dy):
        dyb = dy.astype(BF16)
        ob = o_ref[i]
        do = _dot_nt(wop_ref[...], dyb).reshape(NG, NV, 8, TM)
        dwo_acc[...] += _dot(ob, dyb)
        qp, qn = _phi_t(pq_ref[i].astype(F32))
        phiq = jnp.concatenate([qp, qn], axis=1).astype(BF16)
        rden = rden_ref[layer, i].reshape(NG, 1, 8, TM)
        dden = _hred(do * ob.astype(F32).reshape(NG, NV, 8, TM), jnp.sum, jnp.add) * (-0.5 * rden)
        dna = jnp.concatenate([do * rden, dden, jnp.zeros_like(dden)], axis=1).astype(BF16)
        dphi = []
        for g in range(NG):
            dn = dna[g].reshape(GA, TM)
            dphi.append(_dot(kvm_ref[layer * NG + g], dn))
            kv_acc[g, 0:GF, 0:GA] += _dot_nt(phiq[g].reshape(GF, TM), dn)
        dphi = jnp.concatenate(dphi, axis=0).reshape(NG, 2 * NV, 8, TM)
        dpq = _phi_bwd_t(qp, qn, dphi[:, 0:NV], dphi[:, NV:2 * NV]).reshape(D, TM).astype(BF16)
        h = hs_ref[2 * layer, rows(i), :]
        gout_ref[rows(i), :] = _dot_tn(dpq, wp_ref[0:D, :]).astype(BF16)
        dwp_ref[0:D, :] += _dot(dpq, h)

    def a_bwd2(layer, i, dxp):
        v = v_ref[i]
        kp, kn = _phi_t(pk_ref[i].astype(F32))
        phik = jnp.concatenate([kp, kn], axis=1).astype(BF16)
        dphi, dvs = [], []
        for g in range(NG):
            va = jnp.concatenate([v[g * GR:(g + 1) * GR], ones_rows()], axis=0)
            dphi.append(_dot(dkvm_ref[g], va))
            dvs.append(_dot(dkvt_ref[g], phik[g].reshape(GF, TM)))
        dphi = jnp.concatenate(dphi, axis=0).reshape(NG, 2 * NV, 8, TM)
        dpk = _phi_bwd_t(kp, kn, dphi[:, 0:NV], dphi[:, NV:2 * NV]).reshape(D, TM)
        dkv = jnp.concatenate([dpk] + dvs, axis=0).astype(BF16)
        h = hs_ref[2 * layer, rows(i), :]
        dh = _dot_tn(dkv, wp_ref[D:3 * D, :]) + gout_ref[rows(i), :].astype(F32)
        dwp_ref[D:3 * D, :] += _dot(dkv, h)
        return dxp + _ln_bwd(dh, h.astype(F32), rs_ref[2 * layer, rows(i), :])

    def loop(body, name="loop", unroll=1):
        def b(i, c):
            for k in range(unroll):
                body(i * unroll + k)
            return c
        with jax.named_scope(name):
            lax.fori_loop(0, NB // unroll, b, 0)

    def stage_out(i, val, dst_hbm, stage, semoff):
        slot = i % 2

        @pl.when(i >= 2)
        def _():
            pltpu.make_async_copy(stage.at[slot], dst_hbm.at[rows(i - 2)],
                                  sem_blk.at[semoff + slot]).wait()
        stage[slot] = val
        pltpu.make_async_copy(stage.at[slot], dst_hbm.at[rows(i)], sem_blk.at[semoff + slot]).start()

    def stage_drain(dst_hbm, stage, semoff):
        for i in (NB - 2, NB - 1):
            slot = i % 2
            pltpu.make_async_copy(stage.at[slot], dst_hbm.at[rows(i)],
                                  sem_blk.at[semoff + slot]).wait()

    with jax.named_scope("pre1"):
        in_copies[0].wait()
        kv_acc[...] = jnp.zeros_like(kv_acc)
    with jax.named_scope("P1"):
        a_fwd1x(0, 0)

        def p1(i, c):
            a_fwd1y(i)
            a_fwd1x(0, i + 1)
            return c
        lax.fori_loop(0, NB - 1, p1, 0)
        a_fwd1y(NB - 1)

    with jax.named_scope("pre2"):
        a_fwd_finish(0)
        in_copies[4].wait()

    def p2(layer, name):
        with jax.named_scope(name):
            a_fwd2(layer, 0)

            def body(i, c):
                x1 = xs_ref[1, rows(i), :]
                a_fwd2(layer, i + 1)
                b_fwd1(layer, i, x1)
                return c
            lax.fori_loop(0, NB - 1, body, 0)
            b_fwd1(layer, NB - 1, xs_ref[1, rows(NB - 1), :])
    p2(0, "P2")

    with jax.named_scope("pre3"):
        in_copies[6].wait()
        in_copies[7].wait()
        for k in range(3):
            spill_wait(k)
        kv_acc[...] = jnp.zeros_like(kv_acc)

    with jax.named_scope("P3"):
        xs_ref[0, rows(0), :] = b_fwd2(0, 0)
        a_fwd1x(1, 0)

        def p3(i, c):
            a_fwd1y(i)
            xs_ref[0, rows(i + 1), :] = b_fwd2(0, i + 1)
            a_fwd1x(1, i + 1)
            return c
        lax.fori_loop(0, NB - 1, p3, 0)
        a_fwd1y(NB - 1)

    with jax.named_scope("pre4"):
        a_fwd_finish(1)
        spill_wait(3)
        spill_wait(4)
    p2(1, "P4")

    with jax.named_scope("pre5"):
        spill_wait(5)
        in_copies[8].wait()

    def p5(i):
        gl = _gelu_and_grad(u_ref[rows(i), 0:FH].astype(F32))
        x4 = b_fwd2(1, i, gl)
        stage_out(i, x4, out_hbm.at[0], ostage, NB)
        dy = gout_ref[rows(i), :].astype(F32)
        dx_ref[rows(i), :] = dy
        b_bwd1(1, i, dy, gl)
    loop(p5, "P5", 2)

    with jax.named_scope("pre6"):
        stage_drain(out_hbm.at[0], ostage, NB)
        restore_copy(5).start()
        kv_acc[...] = jnp.zeros_like(kv_acc)

    def p6(layer, name):
        with jax.named_scope(name):
            dz_buf[0] = b_bwd2x(layer, 0)

            def step(i, slot, last):
                dz2 = dz_buf[slot]
                if not last:
                    dzn = b_bwd2x(layer, i + 1)
                dx3 = b_bwd2(layer, i, dx_ref[rows(i), :], dz2)
                dx_ref[rows(i), :] = dx3
                if layer == 1:
                    restore_u_copy(i).start()
                a_bwd1(layer, i, dx3)
                if not last:
                    dz_buf[1 - slot] = dzn

            def body(i, c):
                step(i, i % 2, False)
                return c
            lax.fori_loop(0, NB - 1, body, 0)
            step(NB - 1, (NB - 1) % 2, True)
    p6(1, "P6")

    with jax.named_scope("pre7"):
        a_bwd_finish()
        restore_copy(0).start()
        restore_copy(3).start()
        restore_copy(5).wait()
        for i in range(NB):
            restore_u_copy(i).wait()

    def p7(i):
        dx2 = a_bwd2(1, i, dx_ref[rows(i), :])
        dx_ref[rows(i), :] = dx2
        b_bwd1(0, i, dx2)
    loop(p7, "P7")

    db_copy = pltpu.make_async_copy(dbstage, dbsp_hbm, sem_out.at[0])
    with jax.named_scope("pre8"):
        restore_copy(1).start()
        restore_copy(2).start()
        restore_copy(0).wait()
        restore_copy(3).wait()
        kv_acc[...] = jnp.zeros_like(kv_acc)
    p6(0, "P8")

    def dwqkv_copy(t):
        return pltpu.make_async_copy(wqkv_ref.at[:, t * D:(t + 1) * D],
                                     dwqkv_hbm.at[:, t * D:(t + 1) * D], sem_out.at[6 + t])

    def unfold(t):
        m_ref = phip_ref if t < 2 else pmt_ref
        for j in range(5):
            r0, r1 = RR[j]
            wqkv_ref[:, t * D + 128 * j:t * D + 128 * (j + 1)] = _dot_tn(
                wp_ref[t * D + r0:t * D + r1, :],
                m_ref[r0:r1, 128 * j:128 * (j + 1)]).astype(BF16)
        dwqkv_copy(t).start()

    dwin_copy = pltpu.make_async_copy(win_ref, dwin_hbm, sem_out.at[1])
    dwout_copy = pltpu.make_async_copy(wout_ref, dwout_hbm, sem_out.at[2])
    dwo_copy = pltpu.make_async_copy(wo_ref, dwo_hbm, sem_out.at[3])
    with jax.named_scope("pre9"):
        a_bwd_finish()
        win_ref[...] = dwin_acc[...].astype(BF16)
        dwin_copy.start()
        wout_ref[...] = dwout_acc[...].astype(BF16)
        dwout_copy.start()
        wop_ref[...] = dwo_acc[...].astype(BF16)
        for j in range(5):
            r0, r1 = RR[j]
            wo_ref[128 * j:128 * (j + 1), :] = _dot_tn(
                pmt_ref[r0:r1, 128 * j:128 * (j + 1)], wop_ref[r0:r1, :]).astype(BF16)
        dwo_copy.start()
        wp_ref[0:D, :] = dwp_ref[0:D, :].astype(BF16)
        dwo_acc[...] = jnp.zeros_like(dwo_acc)
        for g in range(SG):
            dwo_acc[g * SR:(g + 1) * SR, KS[g]:KS[g] + 256] = _dot(
                wp_ref[g * SR:(g + 1) * SR, :], wqkv_ref[:, KS[g]:KS[g] + 256])
        unfold(0)
        restore_copy(1).wait()
        restore_copy(2).wait()

    def p9(i):
        dgb = dg_ref[rows(i), :]
        dwsp = _dot_nt(dgb, z2_ref[...]).astype(BF16)
        db = _dot_nt(jnp.ones((8, 2 * FH), BF16), dgb)
        dx0 = a_bwd2(0, i, dx_ref[rows(i), :])
        stage_out(i, dwsp, dwsp_hbm, wspstage, NB + 2)
        dbstage[:, pl.ds(pl.multiple_of(i * TM, TM), TM)] = db[0:1, :].astype(BF16)
        stage_out(i, dx0.astype(BF16), dx_hbm.at[0], ostage, NB)
    loop(p9, "P9")

    dwphi_copy = pltpu.make_async_copy(dwphi_stage, dwphi_hbm, sem_out.at[5])
    with jax.named_scope("final"):
        db_copy.start()
        wp_ref[D:3 * D, :] = dwp_ref[D:3 * D, :].astype(BF16)
        unfold(2)
        for g in range(SG):
            dwo_acc[g * SR:(g + 1) * SR, KS[g]:KS[g] + 256] += _dot(
                wp_ref[D + g * SR:D + (g + 1) * SR, :], wqkv_ref[:, D + KS[g]:D + KS[g] + 256])
        unfold(1)
        mm = jnp.where(head_mask(), dwo_acc[...], 0.0)
        mhi = mm.astype(BF16)
        mlo = (mm - mhi.astype(F32)).astype(BF16)
        wphi2_ref[...] = _dot_tn(mhi, et_mat()) + _dot_tn(mlo, et_mat())
        for hh in range(H):
            dwphi_stage[hh] = wphi2_ref[hh * DH:(hh + 1) * DH, :].astype(BF16)
        dwphi_copy.start()

    with jax.named_scope("drain"):
        stage_drain(dwsp_hbm, wspstage, NB + 2)
        stage_drain(dx_hbm.at[0], ostage, NB)
        db_copy.wait()
        dwin_copy.wait()
        dwout_copy.wait()
        dwo_copy.wait()
        for t in range(3):
            dwqkv_copy(t).wait()
        dwphi_copy.wait()


@jax.jit
def pallas_interleave_layers__linear_kernel_hedgehog__mixer_gmlp__prompt_kernel(
    A_x: jax.Array,
    A_wqkv: jax.Array,
    A_w_phi: jax.Array,
    A_wo: jax.Array,
    B_x: jax.Array,
    B_w_in: jax.Array,
    B_w_sp: jax.Array,
    B_b_sp: jax.Array,
    B_w_out: jax.Array,
    grad_out: jax.Array,
):
    del B_x
    bsp2d = B_b_sp.reshape(1, S)

    any_spec = pl.BlockSpec(memory_space=pl.ANY)
    out_shape = (
        jax.ShapeDtypeStruct((1, S, D), BF16),
        jax.ShapeDtypeStruct((1, S, D), BF16),
        jax.ShapeDtypeStruct((D, 3 * D), BF16),
        jax.ShapeDtypeStruct((H, DH, DH), BF16),
        jax.ShapeDtypeStruct((D, D), BF16),
        jax.ShapeDtypeStruct((D, F2), BF16),
        jax.ShapeDtypeStruct((S, S), BF16),
        jax.ShapeDtypeStruct((1, S), BF16),
        jax.ShapeDtypeStruct((FH, D), BF16),
        jax.ShapeDtypeStruct((NB, D, TM), BF16),
        jax.ShapeDtypeStruct((NB, D, TM), BF16),
        jax.ShapeDtypeStruct((NB, D, TM), BF16),
        jax.ShapeDtypeStruct((NB, D, TM), BF16),
        jax.ShapeDtypeStruct((S, F2), BF16),
        jax.ShapeDtypeStruct((S, FH), BF16),
    )
    scratch_shapes = [
        pltpu.VMEM((2, S, D), BF16),
        pltpu.VMEM((4, S, D), BF16),
        pltpu.VMEM((4, S, 1), F32),
        pltpu.VMEM((S, D), BF16),
        pltpu.VMEM((S, D), F32),
        pltpu.VMEM((NB, D, TM), BF16),
        pltpu.VMEM((NB, D, TM), BF16),
        pltpu.VMEM((NB, D, TM), BF16),
        pltpu.VMEM((NB, D, TM), BF16),
        pltpu.VMEM((S, F2), BF16),
        pltpu.VMEM((S, FH), BF16),
        pltpu.VMEM((S, 2 * FH), BF16),
        pltpu.VMEM((S, 2 * FH), BF16),
        pltpu.VMEM((D, 3 * D), BF16),
        pltpu.VMEM((H, DH, DH), BF16),
        pltpu.VMEM((D, DH), F32),
        pltpu.VMEM((D, D), BF16),
        pltpu.VMEM((D, F2), BF16),
        pltpu.VMEM((S, S), BF16),
        pltpu.VMEM((1, S), BF16),
        pltpu.VMEM((FH, D), BF16),
        pltpu.VMEM((3 * D, D), BF16),
        pltpu.VMEM((D, D), BF16),
        pltpu.VMEM((D, D), BF16),
        pltpu.VMEM((D, D), BF16),
        pltpu.VMEM((S, 128), F32),
        pltpu.VMEM((3 * D, D), F32),
        pltpu.VMEM((D, D), F32),
        pltpu.VMEM((D, F2), F32),
        pltpu.VMEM((FH, D), F32),
        pltpu.VMEM((NG, 256, 128), F32),
        pltpu.VMEM((2 * NG, GF, GA), BF16),
        pltpu.VMEM((2 * NG, GA, GF), BF16),
        pltpu.VMEM((NG, GF, GA), BF16),
        pltpu.VMEM((NG, GR, GF), BF16),
        pltpu.VMEM((2, NB, 8 * NG, TM), F32),
        pltpu.VMEM((2, S, 1), F32),
        pltpu.VMEM((2, TM, FH), F32),
        pltpu.VMEM((2, TM, D), BF16),
        pltpu.VMEM((2, TM, S), BF16),
        pltpu.VMEM((1, S), BF16),
        pltpu.VMEM((H, DH, DH), BF16),
        pltpu.SemaphoreType.DMA((12,)),
        pltpu.SemaphoreType.DMA((6 * NB,)),
        pltpu.SemaphoreType.DMA((6,)),
        pltpu.SemaphoreType.DMA((9,)),
        pltpu.SemaphoreType.DMA((NB + 4,)),
    ]
    outs = pl.pallas_call(
        _kernel,
        out_shape=out_shape,
        in_specs=[any_spec] * 9,
        out_specs=tuple([any_spec] * len(out_shape)),
        scratch_shapes=scratch_shapes,
        compiler_params=pltpu.CompilerParams(
            vmem_limit_bytes=125 * 1024 * 1024,
        ),
    )(A_x, A_wqkv, A_w_phi, A_wo, B_w_in, B_w_sp, bsp2d, B_w_out, grad_out)
    out, dx0, dwqkv, dwphi, dwo, dwin, dwsp, dbsp, dwout = outs[:9]
    return (out, dx0, dwqkv, dwphi, dwo, dwin, dwsp,
            dbsp.reshape(S), dwout)
```

```python
import math

import jax
import jax.numpy as jnp
from jax import lax
import jax.experimental.pallas as pl
import jax.experimental.pallas.tpu as pltpu

S = 2048
D = 640
H = 32
DH = 20
F2 = 1536
FH = 768
NG = 8
GR = 80
GF = 160
GA = GR + 16
NV = DH // 2
SG = 4
SR = 160
KS = (0, 128, 256, 384)
RR = ((0, 160), (0, 320), (160, 480), (320, 640), (480, 640))
TM = 256
NB = S // TM
EPS_LN = 1e-5
EPS_DEN = 1e-6
GELU_C = math.sqrt(2.0 / math.pi)
GELU_A = 0.044715

F32 = jnp.float32
BF16 = jnp.bfloat16


def _dot(a, b):
    return jnp.dot(a, b, preferred_element_type=F32)


def _dot_nt(a, b):
    return lax.dot_general(a, b, (((1,), (1,)), ((), ())), preferred_element_type=F32)


def _dot_tn(a, b):
    return lax.dot_general(a, b, (((0,), (0,)), ((), ())), preferred_element_type=F32)


def _ln(x):
    m = jnp.mean(x, axis=-1, keepdims=True)
    xc = x - m
    v = jnp.mean(xc * xc, axis=-1, keepdims=True)
    r = lax.rsqrt(v + EPS_LN)
    return xc * r, r


def _ln_bwd(dy, xn, r):
    a = jnp.mean(dy, axis=-1, keepdims=True)
    b = jnp.mean(dy * xn, axis=-1, keepdims=True)
    return r * (dy - a - xn * b)


def _iota(shape, dim):
    return lax.broadcasted_iota(jnp.int32, shape, dim)


def _row_map(r):
    g = (r * 205) >> 14
    rem = r - GR * g
    return rem >> 2, 4 * g + (rem & 3)


def _tile(r, n):
    return jnp.concatenate([r] * n, axis=1)


def _hred(x, red, op):
    r = red(x, axis=1)
    r = op(r, pltpu.roll(r, 4, 1))
    return r[:, None]


def _phi_t(pt):
    p4 = pt.reshape(NG, NV, 8, pt.shape[1])
    mx = _hred(p4, jnp.max, jnp.maximum)
    mn = _hred(p4, jnp.min, jnp.minimum)
    ep = jnp.exp(p4 - mx)
    en = jnp.exp(mn - p4)
    sp = _hred(ep, jnp.sum, jnp.add)
    sn = _hred(en, jnp.sum, jnp.add)
    return ep * (1.0 / sp), en * (1.0 / sn)


def _phi_bwd_t(php, phn, dphp, dphn):
    cp = _hred(dphp * php, jnp.sum, jnp.add)
    cn = _hred(dphn * phn, jnp.sum, jnp.add)
    return php * (dphp - cp) - phn * (dphn - cn)


def _gelu(u):
    t = jnp.tanh(u * (GELU_C + (GELU_C * GELU_A) * (u * u)))
    return u * (0.5 + 0.5 * t)


def _gelu_grad_parts(u):
    u2 = u * u
    t = jnp.tanh(u * (GELU_C + (GELU_C * GELU_A) * u2))
    hp = 0.5 + 0.5 * t
    da = hp + (u * (hp * (1.0 - hp))) * (2.0 * GELU_C + (6.0 * GELU_C * GELU_A) * u2)
    return hp, da


def _gelu_and_grad(u):
    hp, da = _gelu_grad_parts(u)
    return u * hp, da


def _kernel(
    x_hbm, wqkv_hbm, wphi_hbm, wo_hbm, win_hbm, wsp_hbm, bsp_hbm, wout_hbm, gout_hbm,
    out_hbm, dx_hbm, dwqkv_hbm, dwphi_hbm, dwo_hbm, dwin_hbm, dwsp_hbm, dbsp_hbm, dwout_hbm,
    sp_pq, sp_pk, sp_v, sp_o, sp_u, sp_g,
    xs_ref,
    hs_ref,
    rs_ref,
    gout_ref,
    dx_ref,
    pq_ref, pk_ref,
    v_ref, o_ref,
    u_ref,
    g_ref,
    z2_ref,
    dg_ref,
    wqkv_ref,
    wphi_ref,
    wphi2_ref,
    wo_ref,
    win_ref,
    wsp_ref,
    bsp_ref,
    wout_ref,
    wp_ref,
    phip_ref,
    pmt_ref,
    wop_ref,
    bcol_ref,
    dwp_ref,
    dwo_acc,
    dwin_acc,
    dwout_acc,
    kv_acc,
    kvm_ref,
    kvt_ref,
    dkvm_ref,
    dkvt_ref,
    rden_ref,
    r2_ref,
    dz_buf,
    ostage,
    wspstage,
    dbstage,
    dwphi_stage,
    sem_in, sem_spill, sem_rest, sem_out, sem_blk,
):
    def rows(i):
        if isinstance(i, int):
            return pl.ds(i * TM, TM)
        return pl.ds(pl.multiple_of(i * TM, TM), TM)

    wq_copies = [
        pltpu.make_async_copy(wqkv_hbm.at[:, t * D:(t + 1) * D], wqkv_ref.at[:, t * D:(t + 1) * D],
                              sem_in.at[9 + t])
        for t in range(3)
    ]
    pltpu.make_async_copy(wphi_hbm, wphi_ref, sem_in.at[2]).start()
    for c in wq_copies:
        c.start()
    in_copies = [
        pltpu.make_async_copy(x_hbm.at[0], xs_ref.at[0], sem_in.at[0]),
        None,
        None,
        pltpu.make_async_copy(wo_hbm, wo_ref, sem_in.at[3]),
        pltpu.make_async_copy(win_hbm, win_ref, sem_in.at[4]),
        pltpu.make_async_copy(bsp_hbm, bsp_ref, sem_in.at[5]),
        pltpu.make_async_copy(wsp_hbm, wsp_ref, sem_in.at[6]),
        pltpu.make_async_copy(wout_hbm, wout_ref, sem_in.at[7]),
        pltpu.make_async_copy(gout_hbm.at[0], gout_ref, sem_in.at[8]),
    ]
    for c in in_copies:
        if c is not None:
            c.start()

    def pmt_mat():
        f, head = _row_map(_iota((D, D), 0))
        return (_iota((D, D), 1) == head * DH + f).astype(BF16)

    def head_mask():
        c_dd = _iota((D, D), 1)
        _, head = _row_map(_iota((D, D), 0))
        hc = head * DH
        return jnp.logical_and(c_dd >= hc, c_dd < hc + DH)

    def et_mat():
        f, _ = _row_map(_iota((D, DH), 0))
        return (_iota((D, DH), 1) == f).astype(BF16)

    with jax.named_scope("prep"):
        dwp_ref[...] = jnp.zeros_like(dwp_ref)
        dwo_acc[...] = jnp.zeros_like(dwo_acc)
        dwin_acc[...] = jnp.zeros_like(dwin_acc)
        dwout_acc[...] = jnp.zeros_like(dwout_acc)
        pltpu.make_async_copy(wphi_hbm, wphi_ref, sem_in.at[2]).wait()
        for hh in range(H):
            wphi2_ref[hh * DH:(hh + 1) * DH, :] = wphi_ref[hh].astype(F32)
        phip_ref[...] = jnp.where(
            head_mask(), _dot_nt(et_mat(), wphi2_ref[...].astype(BF16)), 0.0).astype(BF16)
        pmt_ref[...] = pmt_mat()
        for t in range(3):
            wq_copies[t].wait()
            m_ref = phip_ref if t < 2 else pmt_ref
            for g in range(SG):
                wp_ref[t * D + g * SR:t * D + (g + 1) * SR, :] = _dot_nt(
                    m_ref[g * SR:(g + 1) * SR, KS[g]:KS[g] + 256],
                    wqkv_ref[:, t * D + KS[g]:t * D + KS[g] + 256]).astype(BF16)
        in_copies[5].wait()
        bcol_ref[...] = jnp.transpose(
            jnp.broadcast_to(bsp_ref[...].astype(F32), (128, S)))
        in_copies[3].wait()
        for g in range(SG):
            wop_ref[g * SR:(g + 1) * SR, :] = _dot(
                pmt_ref[g * SR:(g + 1) * SR, KS[g]:KS[g] + 256],
                wo_ref[KS[g]:KS[g] + 256, :]).astype(BF16)

    def kv_masks():
        r = _iota((256, 128), 0)
        c = _iota((256, 128), 1)
        return (r & 3) == (c & 3), c

    def a_fwd_finish(layer):
        same, c = kv_masks()
        keep = jnp.logical_and(same, c < GR + 8)
        for g in range(NG):
            m = kv_acc[g]
            zb = jnp.broadcast_to(m[:, GR:GR + 1], (256, 128))
            aug = jnp.where(keep, jnp.where(c < GR, m, zb), 0.0)
            kvm_ref[layer * NG + g] = aug[0:GF, 0:GA].astype(BF16)
            kvt_ref[layer * NG + g] = jnp.transpose(aug)[0:GA, 0:GF].astype(BF16)

    def a_bwd_finish():
        same, c = kv_masks()
        for g in range(NG):
            m = jnp.where(same, kv_acc[g], 0.0)
            dzc = jnp.sum(jnp.where(c >= GR, m, 0.0), axis=1, keepdims=True)
            mk = jnp.where(c < GR, m, 0.0)
            aug = jnp.where(c == GR, jnp.broadcast_to(dzc, (256, 128)), mk)
            dkvm_ref[g] = aug[0:GF, 0:GA].astype(BF16)
            dkvt_ref[g] = jnp.transpose(mk)[0:GR, 0:GF].astype(BF16)

    def ones_rows():
        return (_iota((GA - GR, TM), 0) == 0).astype(BF16)

    spill_bufs = [(pq_ref, sp_pq), (pk_ref, sp_pk), (v_ref, sp_v), (o_ref, sp_o),
                  (u_ref, sp_u), (g_ref, sp_g)]

    def spill_copy(k, i):
        src, dst = spill_bufs[k]
        idx = i if k < 4 else rows(i)
        return pltpu.make_async_copy(src.at[idx], dst.at[idx], sem_spill.at[k * NB + i])

    def spill_wait(k):
        for i in range(NB):
            spill_copy(k, i).wait()

    def restore_copy(k):
        dst, src = spill_bufs[k]
        return pltpu.make_async_copy(src, dst, sem_rest.at[k])

    def restore_u_copy(i):
        return pltpu.make_async_copy(sp_u.at[rows(i)], u_ref.at[rows(i)], sem_blk.at[i])

    def a_fwd1x(layer, i):
        x = xs_ref[0, rows(i), :].astype(F32)
        xn, r = _ln(x)
        h = xn.astype(BF16)
        hs_ref[2 * layer, rows(i), :] = h
        rs_ref[2 * layer, rows(i), :] = r
        pt = _dot_nt(wp_ref[...], h)
        pq = pt[0:D].astype(BF16)
        pk = pt[D:2 * D].astype(BF16)
        v = pt[2 * D:3 * D].astype(BF16)
        pq_ref[i, 0:D, :] = pq
        pk_ref[i, 0:D, :] = pk
        v_ref[i] = v
        if layer == 0:
            spill_copy(2, i).start()

    def a_fwd1y(layer, i):
        v = v_ref[i]
        kp, kn = _phi_t(pk_ref[i, 0:D, :].astype(F32))
        phik = jnp.concatenate([kp, kn], axis=1).astype(BF16)
        pk_ref[i] = phik.reshape(2 * D, TM)
        if layer == 0:
            spill_copy(1, i).start()
        for g in range(NG):
            va = jnp.concatenate([v[g * GR:(g + 1) * GR], ones_rows()], axis=0)
            kv_acc[g, 0:GF, 0:GA] += _dot_nt(phik[g].reshape(GF, TM), va)

    def a_fwd2(layer, i):
        x = xs_ref[0, rows(i), :].astype(F32)
        qp, qn = _phi_t(pq_ref[i, 0:D, :].astype(F32))
        phiq = jnp.concatenate([qp, qn], axis=1).astype(BF16)
        pq_ref[i] = phiq.reshape(2 * D, TM)
        if layer == 0:
            spill_copy(0, i).start()
        os_, rds = [], []
        for g in range(NG):
            res = _dot(kvt_ref[layer * NG + g], phiq[g].reshape(GF, TM))
            rd = 1.0 / (res[GR:GR + 8] + EPS_DEN)
            rds.append(rd)
            os_.append(res[0:GR].reshape(NV, 8, TM) * rd[None])
        rden_ref[layer, i] = jnp.concatenate(rds, axis=0)
        o = jnp.concatenate(os_, axis=0).reshape(D, TM).astype(BF16)
        o_ref[i] = o
        if layer == 0:
            spill_copy(3, i).start()
        x1 = (x + _dot_tn(o, wop_ref[...])).astype(BF16)
        xs_ref[1, rows(i), :] = x1

    def b_fwd1(layer, i, x1):
        xn, r = _ln(x1.astype(F32))
        h = xn.astype(BF16)
        hs_ref[2 * layer + 1, rows(i), :] = h
        rs_ref[2 * layer + 1, rows(i), :] = r
        u = _dot(h, win_ref[...]).astype(BF16)
        u_ref[rows(i), :] = u
        if layer == 0:
            spill_copy(4, i).start()
        a2 = _gelu(u[:, FH:F2].astype(F32))
        z2, r2 = _ln(a2)
        z2_ref[rows(i), layer * FH:(layer + 1) * FH] = z2.astype(BF16)
        r2_ref[layer, rows(i), :] = r2

    def b_fwd2(layer, i, gl=None):
        x1 = xs_ref[1, rows(i), :].astype(F32)
        g = _dot(wsp_ref[rows(i), :], z2_ref[:, layer * FH:(layer + 1) * FH])
        g = (g + _tile(bcol_ref[rows(i), :], FH // 128)).astype(BF16)
        g_ref[rows(i), :] = g
        if layer == 0:
            spill_copy(5, i).start()
        z1 = _gelu(u_ref[rows(i), 0:FH].astype(F32)) if gl is None else gl[0]
        y = (z1 * g.astype(F32)).astype(BF16)
        x2 = (x1 + _dot(y, wout_ref[...])).astype(BF16)
        return x2

    def b_bwd1(layer, i, dy, gl=None):
        dyb = dy.astype(BF16)
        g = g_ref[rows(i), :].astype(F32)
        z1, dgelu1 = _gelu_and_grad(u_ref[rows(i), 0:FH].astype(F32)) if gl is None else gl
        y = (z1 * g).astype(BF16)
        dzg = _dot_nt(dyb, wout_ref[...])
        dwout_acc[...] += _dot_tn(y, dyb)
        dg = (dzg * z1).astype(BF16)
        dg_ref[rows(i), layer * FH:(layer + 1) * FH] = dg
        du1 = (dzg * g * dgelu1).astype(BF16)
        h = hs_ref[2 * layer + 1, rows(i), :]
        gout_ref[rows(i), :] = _dot_nt(du1, win_ref[:, 0:FH]).astype(BF16)
        dwin_acc[:, 0:FH] += _dot_tn(h, du1)

    def b_bwd2x(layer, i):
        return _dot_tn(wsp_ref[:, rows(i)], dg_ref[:, layer * FH:(layer + 1) * FH])

    def b_bwd2(layer, i, dxp, dz2):
        _, dgelu2 = _gelu_grad_parts(u_ref[rows(i), FH:F2].astype(F32))
        z2n = z2_ref[rows(i), layer * FH:(layer + 1) * FH].astype(F32)
        du2 = (_ln_bwd(dz2, z2n, r2_ref[layer, rows(i), :]) * dgelu2).astype(BF16)
        h = hs_ref[2 * layer + 1, rows(i), :]
        dh = _dot_nt(du2, win_ref[:, FH:F2]) + gout_ref[rows(i), :].astype(F32)
        dwin_acc[:, FH:F2] += _dot_tn(h, du2)
        return dxp + _ln_bwd(dh, h.astype(F32), rs_ref[2 * layer + 1, rows(i), :])

    def a_bwd1(layer, i, dy):
        dyb = dy.astype(BF16)
        ob = o_ref[i]
        do = _dot_nt(wop_ref[...], dyb).reshape(NG, NV, 8, TM)
        dwo_acc[...] += _dot(ob, dyb)
        phiq = pq_ref[i].reshape(NG, 2 * NV, 8, TM)
        qp = phiq[:, 0:NV].astype(F32)
        qn = phiq[:, NV:2 * NV].astype(F32)
        rden = rden_ref[layer, i].reshape(NG, 1, 8, TM)
        dden = _hred(do * ob.astype(F32).reshape(NG, NV, 8, TM), jnp.sum, jnp.add) * (-0.5 * rden)
        dna = jnp.concatenate([do * rden, dden, jnp.zeros_like(dden)], axis=1).astype(BF16)
        dphi = []
        for g in range(NG):
            dn = dna[g].reshape(GA, TM)
            dphi.append(_dot(kvm_ref[layer * NG + g], dn))
            kv_acc[g, 0:GF, 0:GA] += _dot_nt(phiq[g].reshape(GF, TM), dn)
        dphi = jnp.concatenate(dphi, axis=0).reshape(NG, 2 * NV, 8, TM)
        dpq = _phi_bwd_t(qp, qn, dphi[:, 0:NV], dphi[:, NV:2 * NV]).reshape(D, TM).astype(BF16)
        h = hs_ref[2 * layer, rows(i), :]
        gout_ref[rows(i), :] = _dot_tn(dpq, wp_ref[0:D, :]).astype(BF16)
        dwp_ref[0:D, :] += _dot(dpq, h)

    def a_bwd2(layer, i, dxp):
        v = v_ref[i]
        phik = pk_ref[i].reshape(NG, 2 * NV, 8, TM)
        kp = phik[:, 0:NV].astype(F32)
        kn = phik[:, NV:2 * NV].astype(F32)
        dphi, dvs = [], []
        for g in range(NG):
            va = jnp.concatenate([v[g * GR:(g + 1) * GR], ones_rows()], axis=0)
            dphi.append(_dot(dkvm_ref[g], va))
            dvs.append(_dot(dkvt_ref[g], phik[g].reshape(GF, TM)))
        dphi = jnp.concatenate(dphi, axis=0).reshape(NG, 2 * NV, 8, TM)
        dpk = _phi_bwd_t(kp, kn, dphi[:, 0:NV], dphi[:, NV:2 * NV]).reshape(D, TM)
        dkv = jnp.concatenate([dpk] + dvs, axis=0).astype(BF16)
        h = hs_ref[2 * layer, rows(i), :]
        dh = _dot_tn(dkv, wp_ref[D:3 * D, :]) + gout_ref[rows(i), :].astype(F32)
        dwp_ref[D:3 * D, :] += _dot(dkv, h)
        return dxp + _ln_bwd(dh, h.astype(F32), rs_ref[2 * layer, rows(i), :])

    def loop(body, name="loop", unroll=1):
        def b(i, c):
            for k in range(unroll):
                body(i * unroll + k)
            return c
        with jax.named_scope(name):
            lax.fori_loop(0, NB // unroll, b, 0)

    def stage_out(i, val, dst_hbm, stage, semoff):
        slot = i % 2

        @pl.when(i >= 2)
        def _():
            pltpu.make_async_copy(stage.at[slot], dst_hbm.at[rows(i - 2)],
                                  sem_blk.at[semoff + slot]).wait()
        stage[slot] = val
        pltpu.make_async_copy(stage.at[slot], dst_hbm.at[rows(i)], sem_blk.at[semoff + slot]).start()

    def stage_drain(dst_hbm, stage, semoff):
        for i in (NB - 2, NB - 1):
            slot = i % 2
            pltpu.make_async_copy(stage.at[slot], dst_hbm.at[rows(i)],
                                  sem_blk.at[semoff + slot]).wait()

    with jax.named_scope("pre1"):
        in_copies[0].wait()
        kv_acc[...] = jnp.zeros_like(kv_acc)
    with jax.named_scope("P1"):
        a_fwd1x(0, 0)

        def p1(i, c):
            a_fwd1y(0, i)
            a_fwd1x(0, i + 1)
            return c
        lax.fori_loop(0, NB - 1, p1, 0)
        a_fwd1y(0, NB - 1)

    with jax.named_scope("pre2"):
        a_fwd_finish(0)
        in_copies[4].wait()

    def p2(layer, name):
        with jax.named_scope(name):
            a_fwd2(layer, 0)

            def body(i, c):
                x1 = xs_ref[1, rows(i), :]
                a_fwd2(layer, i + 1)
                b_fwd1(layer, i, x1)
                return c
            lax.fori_loop(0, NB - 1, body, 0)
            b_fwd1(layer, NB - 1, xs_ref[1, rows(NB - 1), :])
    p2(0, "P2")

    with jax.named_scope("pre3"):
        in_copies[6].wait()
        in_copies[7].wait()
        for k in range(3):
            spill_wait(k)
        kv_acc[...] = jnp.zeros_like(kv_acc)

    with jax.named_scope("P3"):
        xs_ref[0, rows(0), :] = b_fwd2(0, 0)
        a_fwd1x(1, 0)

        def p3(i, c):
            a_fwd1y(1, i)
            xs_ref[0, rows(i + 1), :] = b_fwd2(0, i + 1)
            a_fwd1x(1, i + 1)
            return c
        lax.fori_loop(0, NB - 1, p3, 0)
        a_fwd1y(1, NB - 1)

    with jax.named_scope("pre4"):
        a_fwd_finish(1)
        spill_wait(3)
        spill_wait(4)
    p2(1, "P4")

    with jax.named_scope("pre5"):
        spill_wait(5)
        in_copies[8].wait()

    def p5(i):
        gl = _gelu_and_grad(u_ref[rows(i), 0:FH].astype(F32))
        x4 = b_fwd2(1, i, gl)
        stage_out(i, x4, out_hbm.at[0], ostage, NB)
        dy = gout_ref[rows(i), :].astype(F32)
        dx_ref[rows(i), :] = dy
        b_bwd1(1, i, dy, gl)
    loop(p5, "P5", 2)

    with jax.named_scope("pre6"):
        stage_drain(out_hbm.at[0], ostage, NB)
        restore_copy(5).start()
        kv_acc[...] = jnp.zeros_like(kv_acc)

    def p6(layer, name):
        with jax.named_scope(name):
            dz_buf[0] = b_bwd2x(layer, 0)

            def step(i, slot, last):
                dz2 = dz_buf[slot]
                if not last:
                    dzn = b_bwd2x(layer, i + 1)
                dx3 = b_bwd2(layer, i, dx_ref[rows(i), :], dz2)
                dx_ref[rows(i), :] = dx3
                if layer == 1:
                    restore_u_copy(i).start()
                a_bwd1(layer, i, dx3)
                if not last:
                    dz_buf[1 - slot] = dzn

            def body(i, c):
                step(i, i % 2, False)
                return c
            lax.fori_loop(0, NB - 1, body, 0)
            step(NB - 1, (NB - 1) % 2, True)
    p6(1, "P6")

    with jax.named_scope("pre7"):
        a_bwd_finish()
        restore_copy(0).start()
        restore_copy(3).start()
        restore_copy(5).wait()
        for i in range(NB):
            restore_u_copy(i).wait()

    def p7(i):
        dx2 = a_bwd2(1, i, dx_ref[rows(i), :])
        dx_ref[rows(i), :] = dx2
        b_bwd1(0, i, dx2)
    loop(p7, "P7")

    db_copy = pltpu.make_async_copy(dbstage, dbsp_hbm, sem_out.at[0])
    with jax.named_scope("pre8"):
        restore_copy(1).start()
        restore_copy(2).start()
        restore_copy(0).wait()
        restore_copy(3).wait()
        kv_acc[...] = jnp.zeros_like(kv_acc)
    p6(0, "P8")

    def dwqkv_copy(t):
        return pltpu.make_async_copy(wqkv_ref.at[:, t * D:(t + 1) * D],
                                     dwqkv_hbm.at[:, t * D:(t + 1) * D], sem_out.at[6 + t])

    def unfold(t):
        m_ref = phip_ref if t < 2 else pmt_ref
        for j in range(5):
            r0, r1 = RR[j]
            wqkv_ref[:, t * D + 128 * j:t * D + 128 * (j + 1)] = _dot_tn(
                wp_ref[t * D + r0:t * D + r1, :],
                m_ref[r0:r1, 128 * j:128 * (j + 1)]).astype(BF16)
        dwqkv_copy(t).start()

    dwin_copy = pltpu.make_async_copy(win_ref, dwin_hbm, sem_out.at[1])
    dwout_copy = pltpu.make_async_copy(wout_ref, dwout_hbm, sem_out.at[2])
    dwo_copy = pltpu.make_async_copy(wo_ref, dwo_hbm, sem_out.at[3])
    with jax.named_scope("pre9"):
        a_bwd_finish()
        win_ref[...] = dwin_acc[...].astype(BF16)
        dwin_copy.start()
        wout_ref[...] = dwout_acc[...].astype(BF16)
        dwout_copy.start()
        wop_ref[...] = dwo_acc[...].astype(BF16)
        for j in range(5):
            r0, r1 = RR[j]
            wo_ref[128 * j:128 * (j + 1), :] = _dot_tn(
                pmt_ref[r0:r1, 128 * j:128 * (j + 1)], wop_ref[r0:r1, :]).astype(BF16)
        dwo_copy.start()
        wp_ref[0:D, :] = dwp_ref[0:D, :].astype(BF16)
        dwo_acc[...] = jnp.zeros_like(dwo_acc)
        for g in range(SG):
            dwo_acc[g * SR:(g + 1) * SR, KS[g]:KS[g] + 256] = _dot(
                wp_ref[g * SR:(g + 1) * SR, :], wqkv_ref[:, KS[g]:KS[g] + 256])
        unfold(0)
        restore_copy(1).wait()
        restore_copy(2).wait()

    def p9(i):
        dgb = dg_ref[rows(i), :]
        dwsp = _dot_nt(dgb, z2_ref[...]).astype(BF16)
        db = _dot_nt(jnp.ones((8, 2 * FH), BF16), dgb)
        dx0 = a_bwd2(0, i, dx_ref[rows(i), :])
        stage_out(i, dwsp, dwsp_hbm, wspstage, NB + 2)
        dbstage[:, pl.ds(pl.multiple_of(i * TM, TM), TM)] = db[0:1, :].astype(BF16)
        stage_out(i, dx0.astype(BF16), dx_hbm.at[0], ostage, NB)
    loop(p9, "P9")

    dwphi_copy = pltpu.make_async_copy(dwphi_stage, dwphi_hbm, sem_out.at[5])
    with jax.named_scope("final"):
        db_copy.start()
        wp_ref[D:3 * D, :] = dwp_ref[D:3 * D, :].astype(BF16)
        unfold(2)
        for g in range(SG):
            dwo_acc[g * SR:(g + 1) * SR, KS[g]:KS[g] + 256] += _dot(
                wp_ref[D + g * SR:D + (g + 1) * SR, :], wqkv_ref[:, D + KS[g]:D + KS[g] + 256])
        unfold(1)
        mm = jnp.where(head_mask(), dwo_acc[...], 0.0)
        mhi = mm.astype(BF16)
        mlo = (mm - mhi.astype(F32)).astype(BF16)
        wphi2_ref[...] = _dot_tn(mhi, et_mat()) + _dot_tn(mlo, et_mat())
        for hh in range(H):
            dwphi_stage[hh] = wphi2_ref[hh * DH:(hh + 1) * DH, :].astype(BF16)
        dwphi_copy.start()

    with jax.named_scope("drain"):
        stage_drain(dwsp_hbm, wspstage, NB + 2)
        stage_drain(dx_hbm.at[0], ostage, NB)
        db_copy.wait()
        dwin_copy.wait()
        dwout_copy.wait()
        dwo_copy.wait()
        for t in range(3):
            dwqkv_copy(t).wait()
        dwphi_copy.wait()


@jax.jit
def pallas_interleave_layers__linear_kernel_hedgehog__mixer_gmlp__prompt_kernel(
    A_x: jax.Array,
    A_wqkv: jax.Array,
    A_w_phi: jax.Array,
    A_wo: jax.Array,
    B_x: jax.Array,
    B_w_in: jax.Array,
    B_w_sp: jax.Array,
    B_b_sp: jax.Array,
    B_w_out: jax.Array,
    grad_out: jax.Array,
):
    del B_x
    bsp2d = B_b_sp.reshape(1, S)

    any_spec = pl.BlockSpec(memory_space=pl.ANY)
    out_shape = (
        jax.ShapeDtypeStruct((1, S, D), BF16),
        jax.ShapeDtypeStruct((1, S, D), BF16),
        jax.ShapeDtypeStruct((D, 3 * D), BF16),
        jax.ShapeDtypeStruct((H, DH, DH), BF16),
        jax.ShapeDtypeStruct((D, D), BF16),
        jax.ShapeDtypeStruct((D, F2), BF16),
        jax.ShapeDtypeStruct((S, S), BF16),
        jax.ShapeDtypeStruct((1, S), BF16),
        jax.ShapeDtypeStruct((FH, D), BF16),
        jax.ShapeDtypeStruct((NB, 2 * D, TM), BF16),
        jax.ShapeDtypeStruct((NB, 2 * D, TM), BF16),
        jax.ShapeDtypeStruct((NB, D, TM), BF16),
        jax.ShapeDtypeStruct((NB, D, TM), BF16),
        jax.ShapeDtypeStruct((S, F2), BF16),
        jax.ShapeDtypeStruct((S, FH), BF16),
    )
    scratch_shapes = [
        pltpu.VMEM((2, S, D), BF16),
        pltpu.VMEM((4, S, D), BF16),
        pltpu.VMEM((4, S, 1), F32),
        pltpu.VMEM((S, D), BF16),
        pltpu.VMEM((S, D), F32),
        pltpu.VMEM((NB, 2 * D, TM), BF16),
        pltpu.VMEM((NB, 2 * D, TM), BF16),
        pltpu.VMEM((NB, D, TM), BF16),
        pltpu.VMEM((NB, D, TM), BF16),
        pltpu.VMEM((S, F2), BF16),
        pltpu.VMEM((S, FH), BF16),
        pltpu.VMEM((S, 2 * FH), BF16),
        pltpu.VMEM((S, 2 * FH), BF16),
        pltpu.VMEM((D, 3 * D), BF16),
        pltpu.VMEM((H, DH, DH), BF16),
        pltpu.VMEM((D, DH), F32),
        pltpu.VMEM((D, D), BF16),
        pltpu.VMEM((D, F2), BF16),
        pltpu.VMEM((S, S), BF16),
        pltpu.VMEM((1, S), BF16),
        pltpu.VMEM((FH, D), BF16),
        pltpu.VMEM((3 * D, D), BF16),
        pltpu.VMEM((D, D), BF16),
        pltpu.VMEM((D, D), BF16),
        pltpu.VMEM((D, D), BF16),
        pltpu.VMEM((S, 128), F32),
        pltpu.VMEM((3 * D, D), F32),
        pltpu.VMEM((D, D), F32),
        pltpu.VMEM((D, F2), F32),
        pltpu.VMEM((FH, D), F32),
        pltpu.VMEM((NG, 256, 128), F32),
        pltpu.VMEM((2 * NG, GF, GA), BF16),
        pltpu.VMEM((2 * NG, GA, GF), BF16),
        pltpu.VMEM((NG, GF, GA), BF16),
        pltpu.VMEM((NG, GR, GF), BF16),
        pltpu.VMEM((2, NB, 8 * NG, TM), F32),
        pltpu.VMEM((2, S, 1), F32),
        pltpu.VMEM((2, TM, FH), F32),
        pltpu.VMEM((2, TM, D), BF16),
        pltpu.VMEM((2, TM, S), BF16),
        pltpu.VMEM((1, S), BF16),
        pltpu.VMEM((H, DH, DH), BF16),
        pltpu.SemaphoreType.DMA((12,)),
        pltpu.SemaphoreType.DMA((6 * NB,)),
        pltpu.SemaphoreType.DMA((6,)),
        pltpu.SemaphoreType.DMA((9,)),
        pltpu.SemaphoreType.DMA((NB + 4,)),
    ]
    outs = pl.pallas_call(
        _kernel,
        out_shape=out_shape,
        in_specs=[any_spec] * 9,
        out_specs=tuple([any_spec] * len(out_shape)),
        scratch_shapes=scratch_shapes,
        compiler_params=pltpu.CompilerParams(
            vmem_limit_bytes=125 * 1024 * 1024,
        ),
    )(A_x, A_wqkv, A_w_phi, A_wo, B_w_in, B_w_sp, bsp2d, B_w_out, grad_out)
    out, dx0, dwqkv, dwphi, dwo, dwin, dwsp, dbsp, dwout = outs[:9]
    return (out, dx0, dwqkv, dwphi, dwo, dwin, dwsp,
            dbsp.reshape(S), dwout)
```
